```python
import jax
import jax.numpy as jnp

def _softmax(x, axis=-1):
    return jax.nn.softmax(x, axis=axis)
def _gelu(x):
    return jax.nn.gelu(x, approximate=True)
def _silu(x):
    return jax.nn.silu(x)
def _sigmoid(x):
    return jax.nn.sigmoid(x)
def _layernorm(x, axis=-1, eps=1e-5):
    m = jnp.mean(x, axis=axis, keepdims=True)
    v = jnp.var(x, axis=axis, keepdims=True)
    return (x - m) / jnp.sqrt(v + eps)
def _scatter_add(tgt, idx, src, axis=0):
    return tgt.at[idx].add(src)
def _segment_sum(src, seg, n):
    return jax.ops.segment_sum(src, seg, n)
class _Rng:
    def __init__(self, key):
        self._k = key
    def _next(self):
        self._k, sub = jax.random.split(self._k)
        return sub
    def normal(self, shape):
        return jax.random.normal(self._next(), shape, dtype=jnp.bfloat16)
    def randint(self, lo, hi, shape):
        return jax.random.randint(self._next(), shape, lo, hi, dtype=jnp.int32)
    def uniform(self, shape, lo=0.0, hi=1.0):
        return jax.random.uniform(self._next(), shape, jnp.bfloat16, lo, hi)
    def permutation(self, n):
        return jax.random.permutation(self._next(), n)


kernel_name = 'standalone__batchnorm__sampling'

def setup_inputs():
    _rng = _Rng(jax.random.key(int.from_bytes(__import__("os").urandom(4), "little")))
    _w = (lambda a: (lambda t: t.astype(jnp.bfloat16) if jnp.issubdtype(t.dtype, jnp.floating) else t)(jnp.asarray(a)))
    B, S, C = 1024, 32, 576
    K = 3
    return {
        "x": _w((lambda *s: _rng.normal(s) * 0.05)(B, S, C)),
        "w": _w((lambda *s: _rng.normal(s) * 0.05)(K, C, C) * (1.0 / (K * C) ** 0.5)),
        "mean": _w((lambda *s: _rng.normal(s) * 0.05)(C) * 0.1),
        "var": _w(jnp.abs((lambda *s: _rng.normal(s) * 0.05)(C)) + 0.5),
        "g": _w((lambda *s: _rng.normal(s) * 0.05)(C) + 1.0),
        "b": _w((lambda *s: _rng.normal(s) * 0.05)(C) * 0.1),
    }

def reference(x, w, mean, var, g, b):
    K = 3
    P = K // 2
    S = x.shape[1]
    xp = jnp.pad(x, ((0, 0), (P, P), (0, 0)))
    y = sum(jnp.einsum('bsc,cd->bsd', xp[:, k:k + S, :], w[k]) for k in range(K))
    inv_std = 1.0 / jnp.sqrt(var + 1e-5)
    y = (y - mean) * (g * inv_std) + b
    return _silu(y)
```

```python
import jax
import jax.numpy as jnp
import jax.experimental.pallas as pl
import jax.experimental.pallas.tpu as pltpu

f32 = jnp.float32
bf16 = jnp.bfloat16
u32 = jnp.uint32

A = 0.6875
Bp = 1.0 / A
TB = 128


def _in_transform(d0, d1, d2, d3, d4, d5):
    a, b = A, Bp
    a2d2 = (a * a) * d2
    p = d4 - (b * b) * d2
    r = d4 - a2d2
    t0 = (d0 - a2d2) + p
    q = a * d3 - b * d1
    s = b * d3 - a * d1
    t5 = (d1 + d5) - (a * a + b * b) * d3
    return t0, p + q, p - q, r + s, r - s, t5


def _pk(v):
    return pltpu.bitcast(v.astype(bf16), u32)


def _upk(v):
    return pltpu.bitcast(v, bf16)


def _kernel(x_ref, w_ref, p_ref, o_ref, u_ref, sh_ref, t_ref):
    S, C, _ = x_ref.shape
    a, b = A, Bp

    @pl.when(pl.program_id(0) == 0)
    def _():
        p = p_ref[...].astype(f32)
        mean, var, g, bb = p[:, 0:1], p[:, 1:2], p[:, 2:3], p[:, 3:4]
        s = g / jnp.sqrt(var + 1e-5)
        sh_ref[...] = jnp.broadcast_to(0.5 * (bb - mean * s), (C, 128))
        sc = 0.5 * s
        g0 = w_ref[0].astype(f32) * sc
        g1 = w_ref[1].astype(f32) * sc
        g2 = w_ref[2].astype(f32) * sc
        na = 1.0 / (2 * a * a * (a * a - b * b))
        nb = 1.0 / (2 * b * b * (b * b - a * a))
        ea = na * g0 + (na * a * a) * g2
        eb = nb * g0 + (nb * b * b) * g2
        u_ref[0] = _pk(g0)
        u_ref[1] = _pk(ea + (na * a) * g1)
        u_ref[2] = _pk(ea - (na * a) * g1)
        u_ref[3] = _pk(eb + (nb * b) * g1)
        u_ref[4] = _pk(eb - (nb * b) * g1)
        u_ref[5] = _pk(g2)

    def silu2(h):
        return (h + h * jnp.tanh(h)).astype(bf16)

    for j in range(S // 4):
        base = 4 * j
        zero = jnp.zeros((C, TB), f32)
        d0 = x_ref[base - 1].astype(f32) if j > 0 else zero
        d5 = x_ref[base + 4].astype(f32) if base + 4 < S else zero
        ts = _in_transform(d0, *[x_ref[base + k].astype(f32) for k in range(4)], d5)
        for i in range(6):
            t_ref[i] = _pk(ts[i])
        sh = sh_ref[...]

        def m(i):
            return jnp.dot(_upk(u_ref[i]), _upk(t_ref[i]), preferred_element_type=f32)

        m1, m2, m3, m4 = m(1), m(2), m(3), m(4)
        P, Q, R, Sx = m1 + m2, a * (m1 - m2), m3 + m4, b * (m3 - m4)
        o_ref[base + 1] = silu2(Q + Sx + sh)
        o_ref[base + 2] = silu2((a * a) * P + (b * b) * R + sh)
        y0p = P + R + sh
        y3p = (a * a) * Q + (b * b) * Sx + sh
        o_ref[base + 0] = silu2(y0p + m(0))
        o_ref[base + 3] = silu2(y3p + m(5))


@jax.jit
def pallas_standalone__batchnorm__sampling_kernel(
    x: jax.Array,
    w: jax.Array,
    mean: jax.Array,
    var: jax.Array,
    g: jax.Array,
    b: jax.Array,
):
    B, S, C = x.shape
    xt = jnp.transpose(x, (1, 2, 0))
    wt = jnp.transpose(w, (0, 2, 1))
    p = jnp.stack([mean, var, g, b], axis=1)
    out = pl.pallas_call(
        _kernel,
        grid=(B // TB,),
        in_specs=[
            pl.BlockSpec((S, C, TB), lambda i: (0, 0, i)),
            pl.BlockSpec((3, C, C), lambda i: (0, 0, 0)),
            pl.BlockSpec((C, 4), lambda i: (0, 0)),
        ],
        out_specs=pl.BlockSpec((S, C, TB), lambda i: (0, 0, i)),
        out_shape=jax.ShapeDtypeStruct((S, C, B), x.dtype),
        scratch_shapes=[
            pltpu.VMEM((6, C // 2, C), u32),
            pltpu.VMEM((C, 128), f32),
            pltpu.VMEM((6, C // 2, TB), u32),
        ],
        compiler_params=pltpu.CompilerParams(
            dimension_semantics=("arbitrary",),
            vmem_limit_bytes=100 * 1024 * 1024,
        ),
    )(xt, wt, p)
    return jnp.transpose(out, (2, 0, 1))
```

```python
import jax
import jax.numpy as jnp
import jax.experimental.pallas as pl
import jax.experimental.pallas.tpu as pltpu

f32 = jnp.float32
bf16 = jnp.bfloat16
u32 = jnp.uint32

A = 0.6875
Bp = 1.0 / A
TB = 128
KM = 512
KH = KM // 2
CH = 16
CE = 48
WCH = 32
SWAP = (0, 1, 1, 0, 0, 1)
USE = {1: ((0, 0, 1), (1, 1, 1)), 2: ((1, 0, 1), (1, 1, -1)), 3: ((0, 1, 1), (1, 1, 1)),
       4: ((0, 0, 1), (1, 0, 1)), 5: ((0, 0, -1), (0, 1, 1)), 6: ((1, 1, 1),), 7: ((0, 0, 1),),
       11: ((0, 0, 1),), 21: ((1, 0, 1),), 12: ((0, 1, 1),), 22: ((1, 1, 1),)}
SEQ_PAIR = (2, 4, 21, 12, 5, 3, 22, 11, 1, 6, 7)
SEQ_0 = (2, 4, 5, 3, 1, 6, 7)
SEQ_5 = (2, 4, 21, 12, 5, 3, 1, 11, 22, 6, 7)
FIRST = ((0, 9), (9, 17), (17, 32))
FIRST_WAIT = (0, 1)
PS, WS, FS = 0, 4, 10
IS = FS + len(FIRST)
OS = IS + 2
NSEM = OS + 2


def _upk(v):
    return pltpu.bitcast(v, bf16)


def _dsm(lo, n):
    return pl.ds(lo if isinstance(lo, int) else pl.multiple_of(lo, n), n)


def _silu2(h):
    return (h + h * jnp.tanh(h)).astype(bf16)


def _dot(l, r):
    return jnp.dot(_upk(l), r, preferred_element_type=f32)


def _kernel(x_hbm, w_hbm, m_hbm, v_hbm, g_hbm, b_hbm, o_hbm,
            wbuf, pm, pv, pg, pb, gt_ref, a_ref, r_ref, sc_ref, sh_ref, xbuf, obuf, z_ref, sem):
    S, C, B = x_hbm.shape
    ND = S // 8
    NS = B // TB
    MH = C // 2
    a, b = A, Bp
    cc = a * a + b * b
    D = 1.0 / (2 * (b * b - a * a))
    a32, r32 = a_ref.bitcast(u32), r_ref.bitcast(u32)

    def x_copy(st, lo, hi, s):
        return pltpu.make_async_copy(
            x_hbm.at[pl.ds(lo, hi - lo), :, _dsm(st * TB, TB)],
            xbuf.at[st % 2, pl.ds(lo, hi - lo)], s)

    def in_copy(st):
        return x_copy(st, 0, S, sem.at[IS + st % 2])

    def out_copy(st, lo, n):
        return pltpu.make_async_copy(
            obuf.at[st % 2, pl.ds(lo, n)],
            o_hbm.at[pl.ds(lo, n), :, _dsm(st * TB, TB)], sem.at[OS + st % 2])

    def out_wait_all(sl):
        pltpu.make_async_copy(obuf.at[sl], obuf.at[sl], sem.at[OS + sl]).wait()

    def wblk_copy(r):
        return pltpu.make_async_copy(w_hbm.at[:, _dsm(r * 128, 128), :],
                                     wbuf.at[:, _dsm(r * 128, 128), :], sem.at[WS + r])

    pcs = [pltpu.make_async_copy(s, d, sem.at[PS + i])
           for i, (s, d) in enumerate(((m_hbm, pm), (v_hbm, pv), (g_hbm, pg), (b_hbm, pb)))]
    fcs = [x_copy(0, lo, hi, sem.at[FS + k]) for k, (lo, hi) in enumerate(FIRST)]
    wrem_copy = pltpu.make_async_copy(w_hbm.at[:, pl.ds(KM, C - KM), :],
                                      wbuf.at[:, pl.ds(KM, C - KM), :], sem.at[WS + 4])
    wdup_copy = pltpu.make_async_copy(w_hbm.at[0, pl.ds(KM, C - KM), :],
                                      wbuf.at[0, pl.ds(C, C - KM), :], sem.at[WS + 5])

    def xpose(r):
        for k in range(3):
            gt_ref[k, r] = pltpu.bitcast(wbuf[k, _dsm(r * 128, 128), :].T, u32)

    def u_rows(r, lo):
        gs = [_upk(gt_ref[k, r, _dsm(lo // 2, WCH // 2), :]).astype(f32) for k in range(3)]
        sc = sc_ref[_dsm(lo, WCH), :]
        scd = sc * D
        ea = ((-b * b) * gs[0] - gs[2]) * scd
        eb = ((a * a) * gs[0] + gs[2]) * scd
        h1 = gs[1] * scd
        return [gs[0] * (-sc), ea - b * h1, ea + b * h1, eb + a * h1, eb - a * h1, gs[2] * sc]

    for c in pcs:
        c.start()
    for r in (0, 2, 1, 3):
        wblk_copy(r).start()
    wrem_copy.start()
    wdup_copy.start()
    for c in fcs:
        c.start()
    in_copy(1).start()
    wbuf[1:3, C:, :] = jnp.zeros((2, C - KM, C), bf16)
    for c in pcs:
        c.wait()
    mean, var, g, bb = (r[...].reshape(1, C).astype(f32) for r in (pm, pv, pg, pb))
    sc_all = 0.5 * g / jnp.sqrt(var + 1e-5)
    sc_ref[...] = jnp.broadcast_to(sc_all, (128, C)).T
    sh = jnp.broadcast_to(0.5 * bb - mean * sc_all, (128, C)).T
    sh_ref[0] = sh
    sh_ref[1] = (b * b) * sh
    sh_ref[2] = (1.0 - b * b) * sh
    sh_ref[3] = (1.0 - a * a) * sh

    def wbody(r, carry):
        for k in range(2):
            z_ref[r + 2 * k] = 0
        wblk_copy(r).wait()
        wblk_copy(r + 2).wait()
        xpose(r)
        xpose(r + 2)

        def cbody(c, carry):
            lo = c * WCH
            u11, u12 = u_rows(r, lo), u_rows(r + 2, lo)
            u21, u22 = u_rows(r, MH + lo), u_rows(r + 2, MH + lo)
            for i in range(6):
                a11, a12, a21, a22 = u11[i], u12[i], u21[i], u22[i]
                for s, v in enumerate((a11 + a22, a21 + a22, a11, a22,
                                       a11 + a12, a21 - a11, a12 - a22)):
                    a_ref[i, s, r, _dsm(lo, WCH), :] = v.astype(bf16)
            return carry

        return jax.lax.fori_loop(0, MH // WCH, cbody, carry)

    jax.lax.fori_loop(0, 2, wbody, 0)
    wrem_copy.wait()
    wdup_copy.wait()
    xpose(4)

    def rbody(c, carry):
        us = u_rows(4, c * WCH)
        for i in range(1, 6):
            r_ref[i - 1, _dsm(c * WCH, WCH), :] = us[i].astype(bf16)
        return carry

    jax.lax.fori_loop(0, C // WCH, rbody, 0)
    fcs[0].wait()

    def block(step, waits, s_ref):
        o_ref = obuf.at[step % 2]
        s32 = s_ref.bitcast(u32)
        chunks = [slice(c * CE, (c + 1) * CE) for c in range(MH // CE)]

        def t_rows(j, rows, grp, cell):
            xb = xbuf.at[(step + z_ref[cell]) & 1]

            def dd(k):
                i = 4 * j - 1 + k
                return xb[i, rows, :].astype(f32) if 0 <= i < S else None

            if grp == (1, 2):
                p = dd(4) - (b * b) * dd(2)
                q = a * dd(3) - b * dd(1)
                return p + q, p - q
            if grp == (3, 4):
                p = dd(4) - (a * a) * dd(2)
                q = b * dd(3) - a * dd(1)
                return p + q, p - q
            if grp == (0,):
                d0 = dd(0)
                return (cc * dd(2) - (dd(4) if d0 is None else dd(4) + d0),)
            d5 = dd(5)
            return ((dd(1) if d5 is None else dd(1) + d5) - cc * dd(3),)

        def to_bf16(v, e, lo):
            n = v.shape[0]
            s_ref[e, lo:lo + n, :] = v.astype(bf16)
            return _upk(s32[e, lo // 2:(lo + n) // 2, :])

        def calc_s(d, grp, cell):
            parts = {i: [[] for _ in range(8)] for i in grp}
            for c in range(KH // CH):
                r1 = slice(c * CH, (c + 1) * CH)
                r2 = slice(KH + c * CH, KH + (c + 1) * CH)
                tl1, tl2 = t_rows(2 * d, r1, grp, cell), t_rows(2 * d, r2, grp, cell)
                tr1, tr2 = t_rows(2 * d + 1, r1, grp, cell), t_rows(2 * d + 1, r2, grp, cell)
                for n, i in enumerate(grp):
                    if SWAP[i]:
                        b11, b21, b12, b22 = tr1[n], tr2[n], tl1[n], tl2[n]
                    else:
                        b11, b21, b12, b22 = tl1[n], tl2[n], tr1[n], tr2[n]
                    for r, v in enumerate((b11 + b22, b11, b12 - b22, b21 - b11,
                                           b22, b11 + b12, b21 + b22)):
                        parts[i][r + 1].append(to_bf16(v, 8 * i + r, c * CH))
            return {i: [None] + [jnp.concatenate(parts[i][r], axis=0) for r in range(1, 8)]
                    for i in grp}

        def calc_rem(d, grp, cell):
            ts = [t_rows(2 * d + X, slice(KM, C), grp, cell) for X in range(2)]
            return {i: [to_bf16(ts[X][n], 8 * i + 7, 64 * X) for X in range(2)]
                    for n, i in enumerate(grp)}

        def orow(h, rows):
            return slice(h * MH + rows.start, h * MH + rows.stop)

        def bias(k, h, rows):
            return sh_ref[k, orow(h, rows), :]

        for d in range(ND):
            def run(prods, cell, seq, on_final):
                ss = calc_s(d, prods, cell)
                if prods != (0,):
                    rem = calc_rem(d, prods, cell)
                    if prods != (5,):
                        rem0 = calc_rem(d, (0,), cell)[0]
                fg = (1, 0) if SWAP[prods[0]] else (0, 1)
                acc, left = {}, {}
                for t in seq:
                    for (h, c, sg) in USE[t]:
                        left[h, c] = left.get((h, c), 0) + 1
                for t in seq:
                    for i in prods:
                        if t < 10:
                            l = jnp.concatenate([a32[i, t - 1, 0], a32[i, t - 1, 1]], axis=1)
                            v = _dot(l, ss[i][t])
                        else:
                            h, X = t // 10 - 1, fg[t % 10 - 1]
                            l = r32[i - 1, h * MH // 2:(h + 1) * MH // 2, :]
                            if i == 5:
                                v = _dot(l[:, :C - KM], rem[i][X])
                            else:
                                v = _dot(l, jnp.concatenate([rem[i][X], rem0[X]], axis=0))
                        for (h, c, sg) in USE[t]:
                            k = (i, h, c)
                            if k not in acc:
                                acc[k] = (v, sg)
                            else:
                                p, ps = acc[k]
                                acc[k] = ((p + v, sg) if ps == sg
                                          else (p - v if ps > 0 else v - p, 1))
                    for (h, c, sg) in USE[t]:
                        left[h, c] -= 1
                        if left[h, c] == 0:
                            on_final(fg[c], h, [acc[i, h, c][0] for i in prods])

            st12, y0p, y3p = {}, {}, {}

            def fin12(X, h, v):
                for c, rows in enumerate(chunks):
                    m1, m2 = v[0][rows], v[1][rows]
                    st12[X, h, c] = ((m1 + m2) + bias(1, h, rows), a * (m1 - m2) + bias(0, h, rows))

            def fin34(X, h, v):
                base = 8 * d + 4 * X
                for c, rows in enumerate(chunks):
                    m3, m4 = v[0][rows], v[1][rows]
                    p, q = st12[X, h, c]
                    r, s = m3 + m4, b * (m3 - m4)
                    o_ref[base + 1, orow(h, rows), :] = _silu2(q + s)
                    o_ref[base + 2, orow(h, rows), :] = _silu2((a * a) * p + (b * b) * r)
                    y0p[X, h, c] = p + r
                    y3p[X, h, c] = (a * a) * q + (b * b) * s

            def fin_last(yp, off, kb):
                def f(X, h, v):
                    for c, rows in enumerate(chunks):
                        o_ref[8 * d + 4 * X + off, orow(h, rows), :] = _silu2(
                            yp[X, h, c] + (v[0][rows] + bias(kb, h, rows)))
                return f

            run((1, 2), 0, SEQ_PAIR, fin12)
            if d in waits:
                waits[d].wait()
            run((3, 4), 1, SEQ_PAIR, fin34)
            run((0,), 2, SEQ_0, fin_last(y0p, 0, 2))
            if d == ND - 1:
                out_copy(step, 8 * d, 3).start()
                out_copy(step, 8 * d + 4, 3).start()
            run((5,), 3, SEQ_5, fin_last(y3p, 3, 3))
            if d == ND - 1:
                out_copy(step, 8 * d + 3, 1).start()
                out_copy(step, 8 * d + 7, 1).start()
            else:
                out_copy(step, 8 * d, 8).start()

    def scoped_block(step, waits):
        pl.run_scoped(lambda s_ref: block(step, waits, s_ref), pltpu.VMEM((48, KH, TB), bf16))

    scoped_block(0, {d: fcs[k + 1] for k, d in enumerate(FIRST_WAIT)})

    def body(step, carry):
        in_copy(step).wait()

        @pl.when(step >= 2)
        def _():
            out_wait_all(step % 2)

        @pl.when(step + 1 < NS)
        def _():
            in_copy(step + 1).start()

        scoped_block(step, {})
        return carry

    jax.lax.fori_loop(1, NS, body, 0)
    out_wait_all(NS % 2)
    out_wait_all((NS - 1) % 2)


@jax.jit
def pallas_standalone__batchnorm__sampling_kernel(
    x: jax.Array,
    w: jax.Array,
    mean: jax.Array,
    var: jax.Array,
    g: jax.Array,
    b: jax.Array,
):
    B, S, C = x.shape
    xt = jnp.transpose(x, (1, 2, 0))
    out = pl.pallas_call(
        _kernel,
        in_specs=[pl.BlockSpec(memory_space=pl.ANY)] * 6,
        out_specs=pl.BlockSpec(memory_space=pl.ANY),
        out_shape=jax.ShapeDtypeStruct((S, C, B), x.dtype),
        scratch_shapes=[pltpu.VMEM((3, C + 64, C), bf16)] + [pltpu.VMEM((C,), bf16)] * 4 + [
            pltpu.VMEM((3, 5, C // 2, 128), u32),
            pltpu.VMEM((6, 7, 2, C // 2, 128), bf16),
            pltpu.VMEM((5, C, 128), bf16),
            pltpu.VMEM((C, 128), f32),
            pltpu.VMEM((4, C, 128), f32),
            pltpu.VMEM((2, S, C, TB), bf16),
            pltpu.VMEM((2, S, C, TB), bf16),
            pltpu.SMEM((4,), jnp.int32),
            pltpu.SemaphoreType.DMA((NSEM,)),
        ],
        compiler_params=pltpu.CompilerParams(
            vmem_limit_bytes=100 * 1024 * 1024,
            disable_bounds_checks=True,
            disable_semaphore_checks=True,
        ),
    )(xt, w, mean, var, g, b)
    return jnp.transpose(out, (2, 0, 1))
```

```python
import jax
import jax.numpy as jnp
import jax.experimental.pallas as pl
import jax.experimental.pallas.tpu as pltpu

f32 = jnp.float32
bf16 = jnp.bfloat16
u32 = jnp.uint32

A = 0.6875
Bp = 1.0 / A
TB = 128
KM = 512
KH = KM // 2
WCH = 16
SWAP = (0, 1, 1, 0, 0, 1)
SDEF = {1: ((1, 1, 1), (2, 2, 1)), 2: ((1, 1, 1),), 3: ((1, 2, 1), (2, 2, -1)),
        4: ((2, 1, 1), (1, 1, -1)), 5: ((2, 2, 1),), 6: ((1, 1, 1), (1, 2, 1)),
        7: ((2, 1, 1), (2, 2, 1))}
USE = {1: ((0, 0, 1), (1, 1, 1)), 2: ((1, 0, 1), (1, 1, -1)), 3: ((0, 1, 1), (1, 1, 1)),
       4: ((0, 0, 1), (1, 0, 1)), 5: ((0, 0, -1), (0, 1, 1)), 6: ((1, 1, 1),), 7: ((0, 0, 1),),
       11: ((0, 0, 1),), 21: ((1, 0, 1),), 12: ((0, 1, 1),), 22: ((1, 1, 1),)}
SEQ_12 = (2, 4, 21, 12, 5, 3, 22, 11, 1, 6, 7)
SEQ_34 = (2, 4, 21, 12, 5, 3, 1, 22, 11, 6, 7)
SEQ_5 = (21, 12, 22, 11, 2, 4, 5, 3, 1, 6, 7)
SEQ_0 = (2, 4, 5, 3, 1, 6, 7)
FIRST = ((0, 5), (5, 9), (9, 17), (17, 32))
PS, WS, FS = 0, 4, 10
IS = FS + len(FIRST)
OS = IS + 2
NSEM = OS + 2


def _upk(v):
    return pltpu.bitcast(v, bf16)


def _dsm(lo, n):
    return pl.ds(lo if isinstance(lo, int) else pl.multiple_of(lo, n), n)


def _silu2(h):
    return (h + h * jnp.tanh(h)).astype(bf16)


def _dot(l, r):
    return jnp.dot(_upk(l), r, preferred_element_type=f32)


def _kernel(x_hbm, w_hbm, m_hbm, v_hbm, g_hbm, b_hbm, o_hbm,
            wbuf, pm, pv, pg, pb, gt_ref, a_ref, r_ref, sc_ref, sh_ref, xbuf, obuf, z_ref, sem):
    S, C, B = x_hbm.shape
    ND = S // 8
    NS = B // TB
    MH = C // 2
    KR = C - KM
    a, b = A, Bp
    cc = a * a + b * b
    D = 1.0 / (2 * (b * b - a * a))
    a32, r32 = a_ref.bitcast(u32), r_ref.bitcast(u32)

    def x_copy(st, lo, hi, s):
        return pltpu.make_async_copy(
            x_hbm.at[pl.ds(lo, hi - lo), :, _dsm(st * TB, TB)],
            xbuf.at[st % 2, pl.ds(lo, hi - lo)], s)

    def in_copy(st):
        return x_copy(st, 0, S, sem.at[IS + st % 2])

    def out_copy(st, lo, n):
        return pltpu.make_async_copy(
            obuf.at[st % 2, pl.ds(lo, n)],
            o_hbm.at[pl.ds(lo, n), :, _dsm(st * TB, TB)], sem.at[OS + st % 2])

    def out_half(st, slab, h):
        return pltpu.make_async_copy(
            obuf.at[st % 2, slab, pl.ds(h * MH, MH)],
            o_hbm.at[slab, pl.ds(h * MH, MH), _dsm(st * TB, TB)], sem.at[OS + st % 2])

    def out_wait_all(sl):
        pltpu.make_async_copy(obuf.at[sl], obuf.at[sl], sem.at[OS + sl]).wait()

    pcs = [pltpu.make_async_copy(s, d, sem.at[PS + i])
           for i, (s, d) in enumerate(((m_hbm, pm), (v_hbm, pv), (g_hbm, pg), (b_hbm, pb)))]
    wcs = [pltpu.make_async_copy(w_hbm.at[:, pl.ds(r * 128, 128), :],
                                 wbuf.at[:, pl.ds(r * 128, 128), :], sem.at[WS + r])
           for r in range(4)]
    wrem_copy = pltpu.make_async_copy(w_hbm.at[:, pl.ds(KM, KR), :],
                                      wbuf.at[:, pl.ds(KM, KR), :], sem.at[WS + 4])
    wdup_copy = pltpu.make_async_copy(w_hbm.at[0, pl.ds(KM, KR), :],
                                      wbuf.at[0, pl.ds(C, KR), :], sem.at[WS + 5])
    fcs = [x_copy(0, lo, hi, sem.at[FS + k]) for k, (lo, hi) in enumerate(FIRST)]

    def xpose(r):
        for k in range(3):
            gt_ref[k, r] = pltpu.bitcast(wbuf[k, pl.ds(r * 128, 128), :].T, u32)

    def u_rows(r, c):
        gs = [_upk(gt_ref[k, r, _dsm(c * (WCH // 2), WCH // 2), :]).astype(f32) for k in range(3)]
        sc = [sc_ref[k, _dsm(c * WCH, WCH), :] for k in range(4)]
        u0 = gs[0] * sc[0]
        u5 = gs[2] * sc[1]
        e = D * u5
        ea = (b * b * D) * u0 - e
        eb = e - (a * a * D) * u0
        hb = gs[1] * sc[2]
        ha = gs[1] * sc[3]
        return [u0, ea - hb, ea + hb, eb + ha, eb - ha, u5]

    def strassen_lhs(r):
        def cbody(c, carry):
            z_ref[(c & 1) + 2 * r] = 0
            u11, u12 = u_rows(r, c), u_rows(r + 2, c)
            u21, u22 = u_rows(r, MH // WCH + c), u_rows(r + 2, MH // WCH + c)
            for i in range(6):
                a11, a12, a21, a22 = u11[i], u12[i], u21[i], u22[i]
                for s, v in enumerate((a11 + a22, a21 + a22, a11, a22,
                                       a11 + a12, a21 - a11, a12 - a22)):
                    a_ref[i, s, r, _dsm(c * WCH, WCH), :] = v.astype(bf16)
            return carry

        jax.lax.fori_loop(0, MH // WCH, cbody, 0)

    def remainder_lhs():
        xpose(4)
        for c in range(C // WCH):
            us = u_rows(4, c)
            for i in range(1, 6):
                r_ref[i - 1, _dsm(c * WCH, WCH), :] = us[i].astype(bf16)

    for c in pcs + [wcs[0], wcs[2], wcs[1], wcs[3], fcs[0], wrem_copy, wdup_copy] + fcs[1:]:
        c.start()
    in_copy(1).start()
    wbuf[1:3, C:, :] = jnp.zeros((2, KR, C), bf16)
    for c in pcs:
        c.wait()
    mean, var, g, bb = (r[...].reshape(1, C).astype(f32) for r in (pm, pv, pg, pb))
    sc_all = 0.5 * g / jnp.sqrt(var + 1e-5)
    scc = jnp.broadcast_to(sc_all, (128, C)).T
    sc_ref[0] = -scc
    sc_ref[1] = scc
    sc_ref[2] = (b * D) * scc
    sc_ref[3] = (a * D) * scc
    sh = jnp.broadcast_to(0.5 * bb - mean * sc_all, (128, C)).T
    sh_ref[0] = sh
    sh_ref[1] = (b * b) * sh
    sh_ref[2] = (1.0 - b * b) * sh
    sh_ref[3] = (1.0 - a * a) * sh
    for r in range(2):
        wcs[r].wait()
        xpose(r)
        wcs[r + 2].wait()
        xpose(r + 2)
        strassen_lhs(r)
    fcs[0].wait()

    def block(step, s_ref):
        first = isinstance(step, int)
        o_ref = obuf.at[step % 2]
        s32 = s_ref.bitcast(u32)

        def t_rows(j, lo, n, grp, cell):
            xb = xbuf.at[(step + z_ref[cell]) & 1]

            def dd(k):
                i = 4 * j - 1 + k
                return xb[i, lo:lo + n, :].astype(f32) if 0 <= i < S else None

            if grp == (1, 2):
                p = dd(4) - (b * b) * dd(2)
                q = a * dd(3) - b * dd(1)
                return p + q, p - q
            if grp == (3, 4):
                p = dd(4) - (a * a) * dd(2)
                q = b * dd(3) - a * dd(1)
                return p + q, p - q
            if grp == (0,):
                d0 = dd(0)
                return (cc * dd(2) - (dd(4) if d0 is None else dd(4) + d0),)
            d5 = dd(5)
            return ((dd(1) if d5 is None else dd(1) + d5) - cc * dd(3),)

        def to_bf16(v, e, lo):
            n = v.shape[0]
            s_ref[e, lo:lo + n, :] = v.astype(bf16)
            return _upk(s32[e, lo // 2:(lo + n) // 2, :])

        class Group:
            def __init__(self, d, prods, cell, seq, on_final):
                self.d, self.prods, self.cell, self.on_final = d, prods, cell, on_final
                self.fg = (1, 0) if SWAP[prods[0]] else (0, 1)
                self.todo = list(seq)
                self.blocks, self.rems, self.acc, self.left, self.ready = {}, {}, {}, {}, []
                for t in seq:
                    for (h, c, _) in USE[t]:
                        self.left[h, c] = self.left.get((h, c), 0) + 1

            def blk(self, k, c):
                if (k, c) not in self.blocks:
                    self.blocks[k, c] = t_rows(2 * self.d + self.fg[c - 1], (k - 1) * KH, KH,
                                               self.prods, self.cell)
                return self.blocks[k, c]

            def rem(self, X):
                if X not in self.rems:
                    j = 2 * self.d + X
                    ts = t_rows(j, KM, KR, self.prods, self.cell)
                    out = [to_bf16(t, 8 * i + 7, KR * X) for i, t in zip(self.prods, ts)]
                    if self.prods != (5,):
                        t0 = to_bf16(t_rows(j, KM, KR, (0,), self.cell)[0], 7, KR * X)
                        out = [jnp.concatenate([o, t0], axis=0) for o in out]
                    self.rems[X] = out
                return self.rems[X]

            def term(self, t):
                self.todo.remove(t)
                for n, i in enumerate(self.prods):
                    if t < 10:
                        vs = [self.blk(k, c)[n] for (k, c, _) in SDEF[t]]
                        if len(vs) == 2:
                            vs = [vs[0] + vs[1] if SDEF[t][1][2] > 0 else vs[0] - vs[1]]
                        l = jnp.concatenate([a32[i, t - 1, 0], a32[i, t - 1, 1]], axis=1)
                        v = _dot(l, to_bf16(vs[0], 8 * i + t - 1, 0))
                    else:
                        h, X = t // 10 - 1, self.fg[t % 10 - 1]
                        l = r32[i - 1, h * MH // 2:(h + 1) * MH // 2, :]
                        v = _dot(l[:, :KR] if i == 5 else l, self.rem(X)[n])
                    for (h, c, sg) in USE[t]:
                        k = (i, h, c)
                        if k not in self.acc:
                            self.acc[k] = (v, sg)
                        else:
                            p, ps = self.acc[k]
                            self.acc[k] = ((p + v, sg) if ps == sg
                                           else (p - v if ps > 0 else v - p, 1))
                for (h, c, _) in USE[t]:
                    self.left[h, c] -= 1
                    if self.left[h, c] == 0:
                        self.ready.append((h, c))

            def flush(self):
                for (h, c) in self.ready:
                    self.on_final(self.fg[c], h, [self.acc[i, h, c][0] for i in self.prods])
                self.ready = []

            def run(self):
                self.flush()
                for t in list(self.todo):
                    self.term(t)
                    self.flush()

        def bias(k, h):
            return sh_ref[k, h * MH:(h + 1) * MH, :]

        for d in range(ND):
            st12, y0p, y3p = {}, {}, {}

            def fin12(X, h, v):
                st12[X, h] = ((v[0] + v[1]) + bias(1, h), a * (v[0] - v[1]) + bias(0, h))

            def fin34(X, h, v):
                p, q = st12[X, h]
                r, s = v[0] + v[1], b * (v[0] - v[1])
                o_ref[8 * d + 4 * X + 1, h * MH:(h + 1) * MH, :] = _silu2(q + s)
                o_ref[8 * d + 4 * X + 2, h * MH:(h + 1) * MH, :] = _silu2((a * a) * p + (b * b) * r)
                y0p[X, h] = p + r
                y3p[X, h] = (a * a) * q + (b * b) * s

            def fin_last(yp, off, kb):
                def f(X, h, v):
                    slab = 8 * d + 4 * X + off
                    o_ref[slab, h * MH:(h + 1) * MH, :] = _silu2(yp[X, h] + (v[0] + bias(kb, h)))
                    if d == ND - 1:
                        out_half(step, slab, h).start()
                return f

            g12 = Group(d, (1, 2), 0, SEQ_12, fin12)
            g34 = Group(d, (3, 4), 1, SEQ_34, fin34)
            g0 = Group(d, (0,), 2, SEQ_0, fin_last(y0p, 0, 2))
            g5 = Group(d, (5,), 3, SEQ_5, fin_last(y3p, 3, 3))
            if first and d == 0:
                for grp in (g12, g34, g5, g0):
                    for t in ((5, 3) if grp.fg[0] else (2, 4)):
                        grp.term(t)
                wrem_copy.wait()
                wdup_copy.wait()
                fcs[1].wait()
                remainder_lhs()
            g12.run()
            if first and d < 2:
                fcs[2 + d].wait()
            g34.run()
            if d == ND - 1:
                out_copy(step, 8 * d + 1, 2).start()
                out_copy(step, 8 * d + 5, 2).start()
            g5.run()
            g0.run()
            if d < ND - 1:
                out_copy(step, 8 * d, 8).start()

    def scoped_block(step):
        pl.run_scoped(lambda s_ref: block(step, s_ref), pltpu.VMEM((48, KH, TB), bf16))

    scoped_block(0)

    def body(step, carry):
        in_copy(step).wait()

        @pl.when(step >= 2)
        def _():
            out_wait_all(step % 2)

        @pl.when(step + 1 < NS)
        def _():
            in_copy(step + 1).start()

        scoped_block(step)
        return carry

    jax.lax.fori_loop(1, NS, body, 0)
    out_wait_all(NS % 2)
    out_wait_all((NS - 1) % 2)


@jax.jit
def pallas_standalone__batchnorm__sampling_kernel(
    x: jax.Array,
    w: jax.Array,
    mean: jax.Array,
    var: jax.Array,
    g: jax.Array,
    b: jax.Array,
):
    B, S, C = x.shape
    xt = jnp.transpose(x, (1, 2, 0))
    out = pl.pallas_call(
        _kernel,
        in_specs=[pl.BlockSpec(memory_space=pl.ANY)] * 6,
        out_specs=pl.BlockSpec(memory_space=pl.ANY),
        out_shape=jax.ShapeDtypeStruct((S, C, B), x.dtype),
        scratch_shapes=[pltpu.VMEM((3, C + 64, C), bf16)] + [pltpu.VMEM((C,), bf16)] * 4 + [
            pltpu.VMEM((3, 5, C // 2, 128), u32),
            pltpu.VMEM((6, 7, 2, C // 2, 128), bf16),
            pltpu.VMEM((5, C, 128), bf16),
            pltpu.VMEM((4, C, 128), f32),
            pltpu.VMEM((4, C, 128), f32),
            pltpu.VMEM((2, S, C, TB), bf16),
            pltpu.VMEM((2, S, C, TB), bf16),
            pltpu.SMEM((4,), jnp.int32),
            pltpu.SemaphoreType.DMA((NSEM,)),
        ],
        compiler_params=pltpu.CompilerParams(
            vmem_limit_bytes=100 * 1024 * 1024,
            disable_bounds_checks=True,
            disable_semaphore_checks=True,
        ),
    )(xt, w, mean, var, g, b)
    return jnp.transpose(out, (2, 0, 1))
```

```python
import jax
import jax.numpy as jnp
import jax.experimental.pallas as pl
import jax.experimental.pallas.tpu as pltpu

f32 = jnp.float32
bf16 = jnp.bfloat16
u32 = jnp.uint32

A = 0.6875
Bp = 1.0 / A
TB = 128
KM = 512
KH = KM // 2
RS = 96
SWAP = (0, 1, 1, 0, 0, 1)
SDEF = {1: ((1, 1, 1), (2, 2, 1)), 2: ((1, 1, 1),), 3: ((1, 2, 1), (2, 2, -1)),
        4: ((2, 1, 1), (1, 1, -1)), 5: ((2, 2, 1),), 6: ((1, 1, 1), (1, 2, 1)),
        7: ((2, 1, 1), (2, 2, 1))}
USE = {1: ((0, 0, 1), (1, 1, 1)), 2: ((1, 0, 1), (1, 1, -1)), 3: ((0, 1, 1), (1, 1, 1)),
       4: ((0, 0, 1), (1, 0, 1)), 5: ((0, 0, -1), (0, 1, 1)), 6: ((1, 1, 1),), 7: ((0, 0, 1),),
       11: ((0, 0, 1),), 21: ((1, 0, 1),), 12: ((0, 1, 1),), 22: ((1, 1, 1),)}
SEQ_12 = (2, 4, 21, 12, 5, 3, 22, 11, 1, 6, 7)
SEQ_34 = (2, 4, 21, 12, 5, 3, 1, 22, 11, 6, 7)
SEQ_5 = (21, 12, 22, 11, 2, 4, 5, 3, 1, 6, 7)
SEQ_0 = (2, 4, 5, 3, 1, 6, 7)
FIRST = ((0, 5), (5, 9), (9, 17), (17, 32))
PS, WS, FS = 0, 4, 10
IS = FS + len(FIRST)
OS = IS + 2
NSEM = OS + 2


def _upk(v):
    return pltpu.bitcast(v, bf16)


def _dsm(lo, n):
    return pl.ds(lo if isinstance(lo, int) else pl.multiple_of(lo, n), n)


def _sl(st):
    return st % 2 if isinstance(st, int) else st & 1


def _silu2(h):
    return (h + h * jnp.tanh(h)).astype(bf16)


def _dot(l, r):
    return jnp.dot(_upk(l), r, preferred_element_type=f32)


def _kernel(x_hbm, w_hbm, m_hbm, v_hbm, g_hbm, b_hbm, o_hbm,
            wbuf, pm, pv, pg, pb, a_ref, r_ref, sc_ref, sh_ref, xbuf, obuf, z_ref, sem):
    S, C, B = x_hbm.shape
    ND = S // 8
    NS = B // TB
    MH = C // 2
    KR = C - KM
    a, b = A, Bp
    cc = a * a + b * b
    D = 1.0 / (2 * (b * b - a * a))
    a32, r32 = a_ref.bitcast(u32), r_ref.bitcast(u32)

    def x_copy(st, lo, hi, s):
        return pltpu.make_async_copy(
            x_hbm.at[pl.ds(lo, hi - lo), :, _dsm(st * TB, TB)],
            xbuf.at[_sl(st), pl.ds(lo, hi - lo)], s)

    def in_copy(st):
        return x_copy(st, 0, S, sem.at[IS + _sl(st)])

    def out_copy(st, lo, n):
        return pltpu.make_async_copy(
            obuf.at[_sl(st), pl.ds(lo, n)],
            o_hbm.at[pl.ds(lo, n), :, _dsm(st * TB, TB)], sem.at[OS + _sl(st)])

    def out_half(st, slab, h):
        return pltpu.make_async_copy(
            obuf.at[_sl(st), slab, pl.ds(h * MH, MH)],
            o_hbm.at[slab, pl.ds(h * MH, MH), _dsm(st * TB, TB)], sem.at[OS + _sl(st)])

    def out_wait_all(sl):
        pltpu.make_async_copy(obuf.at[sl], obuf.at[sl], sem.at[OS + sl]).wait()

    pcs = [pltpu.make_async_copy(s, d, sem.at[PS + i])
           for i, (s, d) in enumerate(((m_hbm, pm), (v_hbm, pv), (g_hbm, pg), (b_hbm, pb)))]

    def w_copy(r):
        return pltpu.make_async_copy(w_hbm.at[:, _dsm(r * 128, 128), :],
                                     wbuf.at[:, _dsm(r * 128, 128), :], sem.at[WS + r])

    wrem_copy = pltpu.make_async_copy(w_hbm.at[:, pl.ds(KM, KR), :],
                                      wbuf.at[:, pl.ds(KM, KR), :], sem.at[WS + 4])
    wdup_copy = pltpu.make_async_copy(w_hbm.at[0, pl.ds(KM, KR), :],
                                      wbuf.at[0, pl.ds(C, KR), :], sem.at[WS + 5])
    fcs = [x_copy(0, lo, hi, sem.at[FS + k]) for k, (lo, hi) in enumerate(FIRST)]

    def u_vals(gs, lo, n):
        sc = [sc_ref[k, lo:lo + n, :] for k in range(4)]
        u0 = gs[0] * sc[0]
        u5 = gs[2] * sc[1]
        e = D * u5
        ea = (b * b * D) * u0 - e
        eb = e - (a * a * D) * u0
        hb = gs[1] * sc[2]
        ha = gs[1] * sc[3]
        return [u0, ea - hb, ea + hb, eb + ha, eb - ha, u5]

    eye = (jax.lax.broadcasted_iota(jnp.int32, (128, 128), 0)
           == jax.lax.broadcasted_iota(jnp.int32, (128, 128), 1)).astype(f32).astype(bf16)

    def tr_rows(k, q, lo, n):
        out = []
        while n > 0:
            t, o = lo // 128, lo % 128
            m = min(n, 128 - o)
            wd = min(128, C - 128 * t)
            w = wbuf[k, _dsm(q * 128, 128), 128 * t:128 * t + wd]
            out.append(jax.lax.dot_general(eye[o:o + m, :wd], w, (((1,), (1,)), ((), ())),
                                           preferred_element_type=f32))
            lo, n = lo + m, n - m
        return out[0] if len(out) == 1 else jnp.concatenate(out, axis=0)

    def strassen_lhs(r, carry):
        z_ref[r] = 0
        z_ref[r + 2] = 0
        w_copy(r).wait()
        w_copy(r + 2).wait()
        for c in range(MH // RS):
            us = {}
            for h in range(2):
                lo = h * MH + c * RS
                gs = [[tr_rows(k, r + 2 * q, lo, RS) for k in range(3)] for q in range(2)]
                for q in range(2):
                    us[h, q] = u_vals(gs[q], lo, RS)
            for i in range(6):
                a11, a12, a21, a22 = us[0, 0][i], us[0, 1][i], us[1, 0][i], us[1, 1][i]
                for s, v in enumerate((a11 + a22, a21 + a22, a11, a22,
                                       a11 + a12, a21 - a11, a12 - a22)):
                    a_ref[i, s, r, c * RS:(c + 1) * RS, :] = v.astype(bf16)
        return carry

    def remainder_lhs():
        us = u_vals([wbuf[k, KM:, :].T.astype(f32) for k in range(3)], 0, C)
        for i in range(1, 6):
            r_ref[i - 1] = us[i].astype(bf16)

    for c in pcs + [w_copy(r) for r in (0, 2, 1, 3)] + [fcs[0], wrem_copy, wdup_copy] + fcs[1:]:
        c.start()
    in_copy(1).start()
    wbuf[1:3, C:, :] = jnp.zeros((2, KR, C), bf16)
    for c in pcs:
        c.wait()
    mean, var, g, bb = (r[...].reshape(1, C).astype(f32) for r in (pm, pv, pg, pb))
    sc_all = 0.5 * g / jnp.sqrt(var + 1e-5)
    scc = jnp.broadcast_to(sc_all, (128, C)).T
    sc_ref[0] = -scc
    sc_ref[1] = scc
    sc_ref[2] = (b * D) * scc
    sc_ref[3] = (a * D) * scc
    sh = jnp.broadcast_to(0.5 * bb - mean * sc_all, (128, C)).T
    sh_ref[0] = sh
    sh_ref[1] = (b * b) * sh
    sh_ref[2] = (1.0 - b * b) * sh
    sh_ref[3] = (1.0 - a * a) * sh
    jax.lax.fori_loop(0, 2, strassen_lhs, 0)
    fcs[0].wait()

    def block(step, s_ref):
        first = isinstance(step, int)
        o_ref = obuf.at[_sl(step)]
        s32 = s_ref.bitcast(u32)

        def t_rows(j, lo, n, grp, cell):
            xb = xbuf.at[(step + z_ref[cell]) & 1]

            def dd(k):
                i = 4 * j - 1 + k
                return xb[i, lo:lo + n, :].astype(f32) if 0 <= i < S else None

            if grp == (1, 2):
                p = dd(4) - (b * b) * dd(2)
                q = a * dd(3) - b * dd(1)
                return p + q, p - q
            if grp == (3, 4):
                p = dd(4) - (a * a) * dd(2)
                q = b * dd(3) - a * dd(1)
                return p + q, p - q
            if grp == (0,):
                d0 = dd(0)
                return (cc * dd(2) - (dd(4) if d0 is None else dd(4) + d0),)
            d5 = dd(5)
            return ((dd(1) if d5 is None else dd(1) + d5) - cc * dd(3),)

        def to_bf16(v, e, lo):
            n = v.shape[0]
            s_ref[e, lo:lo + n, :] = v.astype(bf16)
            return _upk(s32[e, lo // 2:(lo + n) // 2, :])

        class Group:
            def __init__(self, d, prods, cell, seq, on_final):
                self.d, self.prods, self.cell, self.on_final = d, prods, cell, on_final
                self.fg = (1, 0) if SWAP[prods[0]] else (0, 1)
                self.todo = list(seq)
                self.blocks, self.rems, self.rhss = {}, {}, {}
                self.acc, self.left, self.ready = {}, {}, []
                for t in seq:
                    for (h, c, _) in USE[t]:
                        self.left[h, c] = self.left.get((h, c), 0) + 1

            def blk(self, k, c):
                if (k, c) not in self.blocks:
                    self.blocks[k, c] = t_rows(2 * self.d + self.fg[c - 1], (k - 1) * KH, KH,
                                               self.prods, self.cell)
                return self.blocks[k, c]

            def rem(self, X):
                if X not in self.rems:
                    j = 2 * self.d + X
                    ts = t_rows(j, KM, KR, self.prods, self.cell)
                    out = [to_bf16(t, 8 * i + 7, KR * X) for i, t in zip(self.prods, ts)]
                    if self.prods != (5,):
                        t0 = to_bf16(t_rows(j, KM, KR, (0,), self.cell)[0], 7, KR * X)
                        out = [jnp.concatenate([o, t0], axis=0) for o in out]
                    self.rems[X] = out
                return self.rems[X]

            def rhs(self, t, n):
                if (t, n) not in self.rhss:
                    vs = [self.blk(k, c)[n] for (k, c, _) in SDEF[t]]
                    if len(vs) == 2:
                        vs = [vs[0] + vs[1] if SDEF[t][1][2] > 0 else vs[0] - vs[1]]
                    self.rhss[t, n] = to_bf16(vs[0], 8 * self.prods[n] + t - 1, 0)
                return self.rhss[t, n]

            def term(self, t):
                self.todo.remove(t)
                for n, i in enumerate(self.prods):
                    if t < 10:
                        l = jnp.concatenate([a32[i, t - 1, 0], a32[i, t - 1, 1]], axis=1)
                        v = _dot(l, self.rhs(t, n))
                    else:
                        h, X = t // 10 - 1, self.fg[t % 10 - 1]
                        l = r32[i - 1, h * MH // 2:(h + 1) * MH // 2, :]
                        v = _dot(l[:, :KR] if i == 5 else l, self.rem(X)[n])
                    for (h, c, sg) in USE[t]:
                        k = (i, h, c)
                        if k not in self.acc:
                            self.acc[k] = (v, sg)
                        else:
                            p, ps = self.acc[k]
                            self.acc[k] = ((p + v, sg) if ps == sg
                                           else (p - v if ps > 0 else v - p, 1))
                for (h, c, _) in USE[t]:
                    self.left[h, c] -= 1
                    if self.left[h, c] == 0:
                        self.ready.append((h, c))

            def flush(self):
                for (h, c) in self.ready:
                    self.on_final(self.fg[c], h, [self.acc[i, h, c][0] for i in self.prods])
                self.ready = []

            def run(self):
                self.flush()
                for t in list(self.todo):
                    self.term(t)
                    self.flush()

        def bias(k, h):
            return sh_ref[k, h * MH:(h + 1) * MH, :]

        for d in range(ND):
            st12, y0p, y3p = {}, {}, {}

            def fin12(X, h, v):
                st12[X, h] = ((v[0] + v[1]) + bias(1, h), a * (v[0] - v[1]) + bias(0, h))

            def fin34(X, h, v):
                p, q = st12[X, h]
                r, s = v[0] + v[1], b * (v[0] - v[1])
                o_ref[8 * d + 4 * X + 1, h * MH:(h + 1) * MH, :] = _silu2(q + s)
                o_ref[8 * d + 4 * X + 2, h * MH:(h + 1) * MH, :] = _silu2((a * a) * p + (b * b) * r)
                y0p[X, h] = p + r
                y3p[X, h] = (a * a) * q + (b * b) * s

            def fin_last(yp, off, kb):
                def f(X, h, v):
                    slab = 8 * d + 4 * X + off
                    o_ref[slab, h * MH:(h + 1) * MH, :] = _silu2(yp[X, h] + (v[0] + bias(kb, h)))
                    if d == ND - 1:
                        out_half(step, slab, h).start()
                return f

            g12 = Group(d, (1, 2), 0, SEQ_12, fin12)
            g34 = Group(d, (3, 4), 1, SEQ_34, fin34)
            g0 = Group(d, (0,), 2, SEQ_0, fin_last(y0p, 0, 2))
            g5 = Group(d, (5,), 3, SEQ_5, fin_last(y3p, 3, 3))
            if first and d == 0:
                for grp in (g12, g34, g5):
                    for t in ((5, 3) if grp.fg[0] else (2, 4)):
                        grp.term(t)
                g0.rhs(2, 0)
                g0.rhs(4, 0)
                wrem_copy.wait()
                wdup_copy.wait()
                fcs[1].wait()
                remainder_lhs()
                g0.term(2)
                g0.term(4)
            g12.run()
            if first and d < 2:
                t = [t for t in g34.todo if t < 10][0]
                g34.todo.remove(t)
                g34.todo.insert(0, t)
                g34.rhs(t, 0)
                g34.rhs(t, 1)
                fcs[2 + d].wait()
            g34.run()
            if d == ND - 1:
                out_copy(step, 8 * d + 1, 2).start()
                out_copy(step, 8 * d + 5, 2).start()
            g5.run()
            g0.run()
            if d < ND - 1:
                out_copy(step, 8 * d, 8).start()

    def scoped_block(step):
        pl.run_scoped(lambda s_ref: block(step, s_ref), pltpu.VMEM((48, KH, TB), bf16))

    scoped_block(0)

    def body(step, carry):
        in_copy(step).wait()

        @pl.when(step >= 2)
        def _():
            out_wait_all(_sl(step))

        @pl.when(step + 1 < NS)
        def _():
            in_copy(step + 1).start()

        scoped_block(step)
        return carry

    jax.lax.fori_loop(1, NS, body, 0)
    out_wait_all(NS % 2)
    out_wait_all((NS - 1) % 2)


@jax.jit
def pallas_standalone__batchnorm__sampling_kernel(
    x: jax.Array,
    w: jax.Array,
    mean: jax.Array,
    var: jax.Array,
    g: jax.Array,
    b: jax.Array,
):
    B, S, C = x.shape
    xt = jnp.transpose(x, (1, 2, 0))
    out = pl.pallas_call(
        _kernel,
        in_specs=[pl.BlockSpec(memory_space=pl.ANY)] * 6,
        out_specs=pl.BlockSpec(memory_space=pl.ANY),
        out_shape=jax.ShapeDtypeStruct((S, C, B), x.dtype),
        scratch_shapes=[pltpu.VMEM((3, C + 64, C), bf16)] + [pltpu.VMEM((C,), bf16)] * 4 + [
            pltpu.VMEM((6, 7, 2, C // 2, 128), bf16),
            pltpu.VMEM((5, C, 128), bf16),
            pltpu.VMEM((4, C, 128), f32),
            pltpu.VMEM((4, C, 128), f32),
            pltpu.VMEM((2, S, C, TB), bf16),
            pltpu.VMEM((2, S, C, TB), bf16),
            pltpu.SMEM((4,), jnp.int32),
            pltpu.SemaphoreType.DMA((NSEM,)),
        ],
        compiler_params=pltpu.CompilerParams(
            vmem_limit_bytes=100 * 1024 * 1024,
            disable_bounds_checks=True,
            disable_semaphore_checks=True,
        ),
    )(xt, w, mean, var, g, b)
    return jnp.transpose(out, (2, 0, 1))
```

```python
import jax
import jax.numpy as jnp
import jax.experimental.pallas as pl
import jax.experimental.pallas.tpu as pltpu

f32 = jnp.float32
bf16 = jnp.bfloat16
u32 = jnp.uint32

A = 0.6875
Bp = 1.0 / A
TB = 128
KM = 512
KH = KM // 2
RS = 96
SWAP = (0, 1, 1, 0, 0, 1)
SDEF = {1: ((1, 1, 1), (2, 2, 1)), 2: ((1, 1, 1),), 3: ((1, 2, 1), (2, 2, -1)),
        4: ((2, 1, 1), (1, 1, -1)), 5: ((2, 2, 1),), 6: ((1, 1, 1), (1, 2, 1)),
        7: ((2, 1, 1), (2, 2, 1))}
USE = {1: ((0, 0, 1), (1, 1, 1)), 2: ((1, 0, 1), (1, 1, -1)), 3: ((0, 1, 1), (1, 1, 1)),
       4: ((0, 0, 1), (1, 0, 1)), 5: ((0, 0, -1), (0, 1, 1)), 6: ((1, 1, 1),), 7: ((0, 0, 1),),
       11: ((0, 0, 1),), 21: ((1, 0, 1),), 12: ((0, 1, 1),), 22: ((1, 1, 1),)}
SEQ_12 = (2, 4, 21, 12, 5, 3, 22, 11, 1, 6, 7)
SEQ_34 = (2, 4, 21, 12, 5, 3, 1, 22, 11, 6, 7)
SEQ_5 = (21, 12, 22, 11, 2, 4, 5, 3, 1, 6, 7)
SEQ_0 = (2, 4, 5, 3, 1, 6, 7)
FIRST = ((0, 5), (5, 9), (9, 17), (17, 32))
PS, WS, FS = 0, 4, 9
IS = FS + len(FIRST)
OS = IS + 2
NSEM = OS + 2


def _upk(v):
    return pltpu.bitcast(v, bf16)


def _dsm(lo, n):
    return pl.ds(lo if isinstance(lo, int) else pl.multiple_of(lo, n), n)


def _sl(st):
    return st % 2 if isinstance(st, int) else st & 1


def _silu2(h):
    return (h + h * jnp.tanh(h)).astype(bf16)


def _dot(l, r):
    return jnp.dot(_upk(l), r, preferred_element_type=f32)


def _kernel(x_hbm, w_hbm, m_hbm, v_hbm, g_hbm, b_hbm, o_hbm,
            wbuf, pm, pv, pg, pb, a_ref, r_ref, sc_ref, sh_ref, xbuf, obuf, z_ref, sem):
    S, C, B = x_hbm.shape
    ND = S // 8
    NS = B // TB
    MH = C // 2
    KR = C - KM
    a, b = A, Bp
    cc = a * a + b * b
    D = 1.0 / (2 * (b * b - a * a))
    a32, r32 = a_ref.bitcast(u32), r_ref.bitcast(u32)

    def x_copy(st, lo, hi, s):
        return pltpu.make_async_copy(
            x_hbm.at[pl.ds(lo, hi - lo), :, _dsm(st * TB, TB)],
            xbuf.at[_sl(st), pl.ds(lo, hi - lo)], s)

    def in_copy(st):
        return x_copy(st, 0, S, sem.at[IS + _sl(st)])

    def out_copy(st, lo, n):
        return pltpu.make_async_copy(
            obuf.at[_sl(st), pl.ds(lo, n)],
            o_hbm.at[pl.ds(lo, n), :, _dsm(st * TB, TB)], sem.at[OS + _sl(st)])

    def out_half(st, slab, h):
        return pltpu.make_async_copy(
            obuf.at[_sl(st), slab, pl.ds(h * MH, MH)],
            o_hbm.at[slab, pl.ds(h * MH, MH), _dsm(st * TB, TB)], sem.at[OS + _sl(st)])

    def out_wait_all(sl):
        pltpu.make_async_copy(obuf.at[sl], obuf.at[sl], sem.at[OS + sl]).wait()

    pcs = [pltpu.make_async_copy(s, d, sem.at[PS + i])
           for i, (s, d) in enumerate(((m_hbm, pm), (v_hbm, pv), (g_hbm, pg), (b_hbm, pb)))]

    def w_copy(r):
        return pltpu.make_async_copy(w_hbm.at[:, _dsm(r * 128, 128), :],
                                     wbuf.at[:, _dsm(r * 128, 128), :], sem.at[WS + r])

    wrem_copy = pltpu.make_async_copy(w_hbm.at[:, pl.ds(KM, KR), :],
                                      wbuf.at[:, pl.ds(KM, KR), :], sem.at[WS + 4])
    fcs = [x_copy(0, lo, hi, sem.at[FS + k]) for k, (lo, hi) in enumerate(FIRST)]

    def u_vals(gs, lo, n):
        sc = [sc_ref[k, lo:lo + n, :] for k in range(4)]
        u0 = gs[0] * sc[0]
        u5 = gs[2] * sc[1]
        e = D * u5
        ea = (b * b * D) * u0 - e
        eb = e - (a * a * D) * u0
        hb = gs[1] * sc[2]
        ha = gs[1] * sc[3]
        return [u0, ea - hb, ea + hb, eb + ha, eb - ha, u5]

    eye = (jax.lax.broadcasted_iota(jnp.int32, (128, 128), 0)
           == jax.lax.broadcasted_iota(jnp.int32, (128, 128), 1)).astype(f32).astype(bf16)

    def tr_rows(k, q, lo, n):
        out = []
        while n > 0:
            t, o = lo // 128, lo % 128
            m = min(n, 128 - o)
            wd = min(128, C - 128 * t)
            w = wbuf[k, _dsm(q * 128, 128), 128 * t:128 * t + wd]
            out.append(jax.lax.dot_general(eye[o:o + m, :wd], w, (((1,), (1,)), ((), ())),
                                           preferred_element_type=f32))
            lo, n = lo + m, n - m
        return out[0] if len(out) == 1 else jnp.concatenate(out, axis=0)

    def strassen_lhs(r, carry):
        z_ref[r] = 0
        z_ref[r + 2] = 0
        w_copy(r).wait()
        w_copy(r + 2).wait()
        for c in range(MH // RS):
            us = {}
            for h in range(2):
                lo = h * MH + c * RS
                gs = [[tr_rows(k, r + 2 * q, lo, RS) for k in range(3)] for q in range(2)]
                for q in range(2):
                    us[h, q] = u_vals(gs[q], lo, RS)
            for i in range(6):
                a11, a12, a21, a22 = us[0, 0][i], us[0, 1][i], us[1, 0][i], us[1, 1][i]
                for s, v in enumerate((a11 + a22, a21 + a22, a11, a22,
                                       a11 + a12, a21 - a11, a12 - a22)):
                    a_ref[i, s, r, c * RS:(c + 1) * RS, :] = v.astype(bf16)
        return carry

    def remainder_lhs():
        wr = [wbuf[k, KM:, :] for k in range(3)]
        ext = [wr[0], jnp.zeros_like(wr[1]), jnp.zeros_like(wr[2])]
        us = u_vals([jnp.concatenate([wr[k], ext[k]], axis=0).T.astype(f32) for k in range(3)], 0, C)
        for i in range(1, 6):
            r_ref[i - 1] = us[i].astype(bf16)

    for c in pcs + [w_copy(r) for r in (0, 2, 1, 3)] + [fcs[0], wrem_copy] + fcs[1:]:
        c.start()
    in_copy(1).start()
    for c in pcs:
        c.wait()
    mean, var, g, bb = (r[...].reshape(1, C).astype(f32) for r in (pm, pv, pg, pb))
    sc_all = 0.5 * g / jnp.sqrt(var + 1e-5)
    scc = jnp.broadcast_to(sc_all, (128, C)).T
    sc_ref[0] = -scc
    sc_ref[1] = scc
    sc_ref[2] = (b * D) * scc
    sc_ref[3] = (a * D) * scc
    sh = jnp.broadcast_to(0.5 * bb - mean * sc_all, (128, C)).T
    sh_ref[0] = sh
    sh_ref[1] = (b * b) * sh
    sh_ref[2] = (1.0 - b * b) * sh
    sh_ref[3] = (1.0 - a * a) * sh
    jax.lax.fori_loop(0, 2, strassen_lhs, 0)
    fcs[0].wait()

    def block(step, s_ref):
        first = isinstance(step, int)
        o_ref = obuf.at[_sl(step)]
        s32 = s_ref.bitcast(u32)

        def t_rows(j, lo, n, grp, cell):
            xb = xbuf.at[(step + z_ref[cell]) & 1]

            def dd(k):
                i = 4 * j - 1 + k
                return xb[i, lo:lo + n, :].astype(f32) if 0 <= i < S else None

            if grp == (1, 2):
                p = dd(4) - (b * b) * dd(2)
                q = a * dd(3) - b * dd(1)
                return p + q, p - q
            if grp == (3, 4):
                p = dd(4) - (a * a) * dd(2)
                q = b * dd(3) - a * dd(1)
                return p + q, p - q
            if grp == (0,):
                d0 = dd(0)
                return (cc * dd(2) - (dd(4) if d0 is None else dd(4) + d0),)
            d5 = dd(5)
            return ((dd(1) if d5 is None else dd(1) + d5) - cc * dd(3),)

        def to_bf16(v, e, lo):
            n = v.shape[0]
            s_ref[e, lo:lo + n, :] = v.astype(bf16)
            return _upk(s32[e, lo // 2:(lo + n) // 2, :])

        class Group:
            def __init__(self, d, prods, cell, seq, on_final):
                self.d, self.prods, self.cell, self.on_final = d, prods, cell, on_final
                self.fg = (1, 0) if SWAP[prods[0]] else (0, 1)
                self.todo = list(seq)
                self.blocks, self.rems, self.rhss = {}, {}, {}
                self.acc, self.left, self.ready = {}, {}, []
                for t in seq:
                    for (h, c, _) in USE[t]:
                        self.left[h, c] = self.left.get((h, c), 0) + 1

            def blk(self, k, c):
                if (k, c) not in self.blocks:
                    self.blocks[k, c] = t_rows(2 * self.d + self.fg[c - 1], (k - 1) * KH, KH,
                                               self.prods, self.cell)
                return self.blocks[k, c]

            def rem(self, X):
                if X not in self.rems:
                    j = 2 * self.d + X
                    ts = t_rows(j, KM, KR, self.prods, self.cell)
                    out = [to_bf16(t, 8 * i + 7, KR * X) for i, t in zip(self.prods, ts)]
                    if self.prods != (5,):
                        t0 = to_bf16(t_rows(j, KM, KR, (0,), self.cell)[0], 7, KR * X)
                        out = [jnp.concatenate([o, t0], axis=0) for o in out]
                    self.rems[X] = out
                return self.rems[X]

            def rhs(self, t, n):
                if (t, n) not in self.rhss:
                    vs = [self.blk(k, c)[n] for (k, c, _) in SDEF[t]]
                    if len(vs) == 2:
                        vs = [vs[0] + vs[1] if SDEF[t][1][2] > 0 else vs[0] - vs[1]]
                    self.rhss[t, n] = to_bf16(vs[0], 8 * self.prods[n] + t - 1, 0)
                return self.rhss[t, n]

            def term(self, t):
                self.todo.remove(t)
                for n, i in enumerate(self.prods):
                    if t < 10:
                        l = jnp.concatenate([a32[i, t - 1, 0], a32[i, t - 1, 1]], axis=1)
                        v = _dot(l, self.rhs(t, n))
                    else:
                        h, X = t // 10 - 1, self.fg[t % 10 - 1]
                        l = r32[i - 1, h * MH // 2:(h + 1) * MH // 2, :]
                        v = _dot(l[:, :KR] if i == 5 else l, self.rem(X)[n])
                    for (h, c, sg) in USE[t]:
                        k = (i, h, c)
                        if k not in self.acc:
                            self.acc[k] = (v, sg)
                        else:
                            p, ps = self.acc[k]
                            self.acc[k] = ((p + v, sg) if ps == sg
                                           else (p - v if ps > 0 else v - p, 1))
                for (h, c, _) in USE[t]:
                    self.left[h, c] -= 1
                    if self.left[h, c] == 0:
                        self.ready.append((h, c))

            def flush(self):
                for (h, c) in self.ready:
                    self.on_final(self.fg[c], h, [self.acc[i, h, c][0] for i in self.prods])
                self.ready = []

            def run(self):
                self.flush()
                for t in list(self.todo):
                    self.term(t)
                    self.flush()

        def bias(k, h):
            return sh_ref[k, h * MH:(h + 1) * MH, :]

        for d in range(ND):
            st12, y0p, y3p = {}, {}, {}

            def fin12(X, h, v):
                st12[X, h] = ((v[0] + v[1]) + bias(1, h), a * (v[0] - v[1]) + bias(0, h))

            def fin34(X, h, v):
                p, q = st12[X, h]
                r, s = v[0] + v[1], b * (v[0] - v[1])
                o_ref[8 * d + 4 * X + 1, h * MH:(h + 1) * MH, :] = _silu2(q + s)
                o_ref[8 * d + 4 * X + 2, h * MH:(h + 1) * MH, :] = _silu2((a * a) * p + (b * b) * r)
                y0p[X, h] = p + r
                y3p[X, h] = (a * a) * q + (b * b) * s

            def fin_last(yp, off, kb):
                def f(X, h, v):
                    slab = 8 * d + 4 * X + off
                    o_ref[slab, h * MH:(h + 1) * MH, :] = _silu2(yp[X, h] + (v[0] + bias(kb, h)))
                    if d == ND - 1:
                        out_half(step, slab, h).start()
                return f

            g12 = Group(d, (1, 2), 0, SEQ_12, fin12)
            g34 = Group(d, (3, 4), 1, SEQ_34, fin34)
            g0 = Group(d, (0,), 2, SEQ_0, fin_last(y0p, 0, 2))
            g5 = Group(d, (5,), 3, SEQ_5, fin_last(y3p, 3, 3))
            if first and d == 0:
                for grp in (g12, g34, g5):
                    for t in ((5, 3) if grp.fg[0] else (2, 4)):
                        grp.term(t)
                g0.rhs(2, 0)
                g0.rhs(4, 0)
                wrem_copy.wait()
                fcs[1].wait()
                remainder_lhs()
                g0.term(2)
                g0.term(4)
            g12.run()
            if first and d < 2:
                t = [t for t in g34.todo if t < 10][0]
                g34.todo.remove(t)
                g34.todo.insert(0, t)
                g34.rhs(t, 0)
                g34.rhs(t, 1)
                fcs[2 + d].wait()
            g34.run()
            if d == ND - 1:
                out_copy(step, 8 * d + 1, 2).start()
                out_copy(step, 8 * d + 5, 2).start()
            g5.run()
            g0.run()
            if d < ND - 1:
                out_copy(step, 8 * d, 8).start()

    def scoped_block(step):
        pl.run_scoped(lambda s_ref: block(step, s_ref), pltpu.VMEM((48, KH, TB), bf16))

    scoped_block(0)

    def body(step, carry):
        in_copy(step).wait()

        @pl.when(step >= 2)
        def _():
            out_wait_all(_sl(step))

        @pl.when(step + 1 < NS)
        def _():
            in_copy(step + 1).start()

        scoped_block(step)
        return carry

    jax.lax.fori_loop(1, NS, body, 0)
    out_wait_all(NS % 2)
    out_wait_all((NS - 1) % 2)


@jax.jit
def pallas_standalone__batchnorm__sampling_kernel(
    x: jax.Array,
    w: jax.Array,
    mean: jax.Array,
    var: jax.Array,
    g: jax.Array,
    b: jax.Array,
):
    B, S, C = x.shape
    xt = jnp.transpose(x, (1, 2, 0))
    out = pl.pallas_call(
        _kernel,
        in_specs=[pl.BlockSpec(memory_space=pl.ANY)] * 6,
        out_specs=pl.BlockSpec(memory_space=pl.ANY),
        out_shape=jax.ShapeDtypeStruct((S, C, B), x.dtype),
        scratch_shapes=[pltpu.VMEM((3, C, C), bf16)] + [pltpu.VMEM((C,), bf16)] * 4 + [
            pltpu.VMEM((6, 7, 2, C // 2, 128), bf16),
            pltpu.VMEM((5, C, 128), bf16),
            pltpu.VMEM((4, C, 128), f32),
            pltpu.VMEM((4, C, 128), f32),
            pltpu.VMEM((2, S, C, TB), bf16),
            pltpu.VMEM((2, S, C, TB), bf16),
            pltpu.SMEM((4,), jnp.int32),
            pltpu.SemaphoreType.DMA((NSEM,)),
        ],
        compiler_params=pltpu.CompilerParams(
            vmem_limit_bytes=100 * 1024 * 1024,
            disable_bounds_checks=True,
            disable_semaphore_checks=True,
        ),
    )(xt, w, mean, var, g, b)
    return jnp.transpose(out, (2, 0, 1))
```

```python
import jax
import jax.numpy as jnp
import jax.experimental.pallas as pl
import jax.experimental.pallas.tpu as pltpu

f32 = jnp.float32
bf16 = jnp.bfloat16
u32 = jnp.uint32

A = 0.6875
Bp = 1.0 / A
TB = 128
KM = 512
KH = KM // 2
RS = 96
SWAP = (0, 1, 1, 0, 0, 1)
SDEF = {1: ((1, 1, 1), (2, 2, 1)), 2: ((1, 1, 1),), 3: ((1, 2, 1), (2, 2, -1)),
        4: ((2, 1, 1), (1, 1, -1)), 5: ((2, 2, 1),), 6: ((1, 1, 1), (1, 2, 1)),
        7: ((2, 1, 1), (2, 2, 1))}
USE = {1: ((0, 0, 1), (1, 1, 1)), 2: ((1, 0, 1), (1, 1, -1)), 3: ((0, 1, 1), (1, 1, 1)),
       4: ((0, 0, 1), (1, 0, 1)), 5: ((0, 0, -1), (0, 1, 1)), 6: ((1, 1, 1),), 7: ((0, 0, 1),),
       11: ((0, 0, 1),), 21: ((1, 0, 1),), 12: ((0, 1, 1),), 22: ((1, 1, 1),)}
SEQ_12 = (2, 4, 21, 12, 5, 3, 22, 11, 1, 6, 7)
SEQ_34 = (2, 4, 21, 12, 5, 3, 1, 22, 11, 6, 7)
SEQ_5 = (21, 12, 22, 11, 2, 4, 5, 3, 1, 6, 7)
SEQ_0 = (2, 4, 5, 3, 1, 6, 7)
FIRST = ((0, 5), (5, 9), (9, 17), (17, 32))
LATE = ((28, 1), (24, 0))
PS, WS, FS = 0, 4, 9
IS = FS + len(FIRST)
OS = IS + 2
NSEM = OS + 2


def _upk(v):
    return pltpu.bitcast(v, bf16)


def _dsm(lo, n):
    return pl.ds(lo if isinstance(lo, int) else pl.multiple_of(lo, n), n)


def _sl(st):
    return st % 2 if isinstance(st, int) else st & 1


def _silu2(h):
    return (h + h * jnp.tanh(h)).astype(bf16)


def _dot(l, r):
    return jnp.dot(_upk(l), r, preferred_element_type=f32)


def _kernel(x_hbm, w_hbm, m_hbm, v_hbm, g_hbm, b_hbm, o_hbm,
            wbuf, pm, pv, pg, pb, a_ref, r_ref, sc_ref, sh_ref, xbuf, obuf, z_ref, sem):
    S, C, B = x_hbm.shape
    ND = S // 8
    NS = B // TB
    MH = C // 2
    KR = C - KM
    a, b = A, Bp
    cc = a * a + b * b
    D = 1.0 / (2 * (b * b - a * a))
    a32, r32 = a_ref.bitcast(u32), r_ref.bitcast(u32)

    def x_copy(st, lo, hi, s):
        return pltpu.make_async_copy(
            x_hbm.at[pl.ds(lo, hi - lo), :, _dsm(st * TB, TB)],
            xbuf.at[_sl(st), pl.ds(lo, hi - lo)], s)

    def in_copy(st):
        return x_copy(st, 0, S, sem.at[IS + _sl(st)])

    def out_copy(st, lo, n):
        return pltpu.make_async_copy(
            obuf.at[_sl(st), pl.ds(lo, n)],
            o_hbm.at[pl.ds(lo, n), :, _dsm(st * TB, TB)], sem.at[OS + _sl(st)])

    def out_half(st, slab, h):
        return pltpu.make_async_copy(
            obuf.at[_sl(st), slab, pl.ds(h * MH, MH)],
            o_hbm.at[slab, pl.ds(h * MH, MH), _dsm(st * TB, TB)], sem.at[OS + _sl(st)])

    def out_wait_all(sl):
        pltpu.make_async_copy(obuf.at[sl], obuf.at[sl], sem.at[OS + sl]).wait()

    pcs = [pltpu.make_async_copy(s, d, sem.at[PS + i])
           for i, (s, d) in enumerate(((m_hbm, pm), (v_hbm, pv), (g_hbm, pg), (b_hbm, pb)))]

    def w_copy(r):
        return pltpu.make_async_copy(w_hbm.at[:, _dsm(r * 128, 128), :],
                                     wbuf.at[:, _dsm(r * 128, 128), :], sem.at[WS + r])

    wrem_copy = pltpu.make_async_copy(w_hbm.at[:, pl.ds(KM, KR), :],
                                      wbuf.at[:, pl.ds(KM, KR), :], sem.at[WS + 4])
    fcs = [x_copy(0, lo, hi, sem.at[FS + k]) for k, (lo, hi) in enumerate(FIRST)]

    def u_vals(gs, lo, n):
        sc = [sc_ref[k, lo:lo + n, :] for k in range(4)]
        u0 = gs[0] * sc[0]
        u5 = gs[2] * sc[1]
        e = D * u5
        ea = (b * b * D) * u0 - e
        eb = e - (a * a * D) * u0
        hb = gs[1] * sc[2]
        ha = gs[1] * sc[3]
        return [u0, ea - hb, ea + hb, eb + ha, eb - ha, u5]

    eye = (jax.lax.broadcasted_iota(jnp.int32, (128, 128), 0)
           == jax.lax.broadcasted_iota(jnp.int32, (128, 128), 1)).astype(f32).astype(bf16)

    def tr_rows(k, q, lo, n):
        out = []
        while n > 0:
            t, o = lo // 128, lo % 128
            m = min(n, 128 - o)
            wd = min(128, C - 128 * t)
            w = wbuf[k, _dsm(q * 128, 128), 128 * t:128 * t + wd]
            out.append(jax.lax.dot_general(eye[o:o + m, :wd], w, (((1,), (1,)), ((), ())),
                                           preferred_element_type=f32))
            lo, n = lo + m, n - m
        return out[0] if len(out) == 1 else jnp.concatenate(out, axis=0)

    def strassen_lhs(r, carry):
        z_ref[r] = 0
        z_ref[r + 2] = 0
        w_copy(r).wait()
        w_copy(r + 2).wait()
        for c in range(MH // RS):
            us = {}
            for h in range(2):
                lo = h * MH + c * RS
                gs = [[tr_rows(k, r + 2 * q, lo, RS) for k in range(3)] for q in range(2)]
                for q in range(2):
                    us[h, q] = u_vals(gs[q], lo, RS)
            for i in range(6):
                a11, a12, a21, a22 = us[0, 0][i], us[0, 1][i], us[1, 0][i], us[1, 1][i]
                for s, v in enumerate((a11 + a22, a21 + a22, a11, a22,
                                       a11 + a12, a21 - a11, a12 - a22)):
                    a_ref[i, s, r, c * RS:(c + 1) * RS, :] = v.astype(bf16)
        return carry

    def remainder_lhs():
        wr = [wbuf[k, KM:, :] for k in range(3)]
        ext = [wr[0], jnp.zeros_like(wr[1]), jnp.zeros_like(wr[2])]
        us = u_vals([jnp.concatenate([wr[k], ext[k]], axis=0).T.astype(f32) for k in range(3)], 0, C)
        for i in range(1, 6):
            r_ref[i - 1] = us[i].astype(bf16)

    for c in pcs + [w_copy(r) for r in (0, 2, 1, 3)] + [fcs[0], wrem_copy] + fcs[1:]:
        c.start()
    in_copy(1).start()
    for c in pcs:
        c.wait()
    mean, var, g, bb = (r[...].reshape(1, C).astype(f32) for r in (pm, pv, pg, pb))
    sc_all = 0.5 * g / jnp.sqrt(var + 1e-5)
    scc = jnp.broadcast_to(sc_all, (128, C)).T
    sc_ref[0] = -scc
    sc_ref[1] = scc
    sc_ref[2] = (b * D) * scc
    sc_ref[3] = (a * D) * scc
    sh = jnp.broadcast_to(0.5 * bb - mean * sc_all, (128, C)).T
    sh_ref[0] = sh
    sh_ref[1] = (b * b) * sh
    sh_ref[2] = (1.0 - b * b) * sh
    sh_ref[3] = (1.0 - a * a) * sh
    jax.lax.fori_loop(0, 2, strassen_lhs, 0)
    fcs[0].wait()

    def block(step, s_ref):
        first = isinstance(step, int)
        o_ref = obuf.at[_sl(step)]
        s32 = s_ref.bitcast(u32)

        def t_rows(j, lo, n, grp, cell):
            xb = xbuf.at[(step + z_ref[cell]) & 1]

            def dd(k):
                i = 4 * j - 1 + k
                return xb[i, lo:lo + n, :].astype(f32) if 0 <= i < S else None

            if grp == (1, 2):
                p = dd(4) - (b * b) * dd(2)
                q = a * dd(3) - b * dd(1)
                return p + q, p - q
            if grp == (3, 4):
                p = dd(4) - (a * a) * dd(2)
                q = b * dd(3) - a * dd(1)
                return p + q, p - q
            if grp == (0,):
                d0 = dd(0)
                return (cc * dd(2) - (dd(4) if d0 is None else dd(4) + d0),)
            d5 = dd(5)
            return ((dd(1) if d5 is None else dd(1) + d5) - cc * dd(3),)

        def to_bf16(v, e, lo):
            n = v.shape[0]
            s_ref[e, lo:lo + n, :] = v.astype(bf16)
            return _upk(s32[e, lo // 2:(lo + n) // 2, :])

        class Group:
            def __init__(self, d, prods, cell, seq, on_final):
                self.d, self.prods, self.cell, self.on_final = d, prods, cell, on_final
                self.fg = (1, 0) if SWAP[prods[0]] else (0, 1)
                self.todo = list(seq)
                self.blocks, self.rems, self.rhss = {}, {}, {}
                self.acc, self.left, self.ready = {}, {}, []
                for t in seq:
                    for (h, c, _) in USE[t]:
                        self.left[h, c] = self.left.get((h, c), 0) + 1

            def blk(self, k, c):
                if (k, c) not in self.blocks:
                    self.blocks[k, c] = t_rows(2 * self.d + self.fg[c - 1], (k - 1) * KH, KH,
                                               self.prods, self.cell)
                return self.blocks[k, c]

            def rem(self, X):
                if X not in self.rems:
                    j = 2 * self.d + X
                    ts = t_rows(j, KM, KR, self.prods, self.cell)
                    out = [to_bf16(t, 8 * i + 7, KR * X) for i, t in zip(self.prods, ts)]
                    if self.prods != (5,):
                        t0 = to_bf16(t_rows(j, KM, KR, (0,), self.cell)[0], 7, KR * X)
                        out = [jnp.concatenate([o, t0], axis=0) for o in out]
                    self.rems[X] = out
                return self.rems[X]

            def rhs(self, t, n):
                if (t, n) not in self.rhss:
                    vs = [self.blk(k, c)[n] for (k, c, _) in SDEF[t]]
                    if len(vs) == 2:
                        vs = [vs[0] + vs[1] if SDEF[t][1][2] > 0 else vs[0] - vs[1]]
                    self.rhss[t, n] = to_bf16(vs[0], 8 * self.prods[n] + t - 1, 0)
                return self.rhss[t, n]

            def term(self, t):
                self.todo.remove(t)
                for n, i in enumerate(self.prods):
                    if t < 10:
                        l = jnp.concatenate([a32[i, t - 1, 0], a32[i, t - 1, 1]], axis=1)
                        v = _dot(l, self.rhs(t, n))
                    else:
                        h, X = t // 10 - 1, self.fg[t % 10 - 1]
                        l = r32[i - 1, h * MH // 2:(h + 1) * MH // 2, :]
                        v = _dot(l[:, :KR] if i == 5 else l, self.rem(X)[n])
                    for (h, c, sg) in USE[t]:
                        k = (i, h, c)
                        if k not in self.acc:
                            self.acc[k] = (v, sg)
                        else:
                            p, ps = self.acc[k]
                            self.acc[k] = ((p + v, sg) if ps == sg
                                           else (p - v if ps > 0 else v - p, 1))
                for (h, c, _) in USE[t]:
                    self.left[h, c] -= 1
                    if self.left[h, c] == 0:
                        self.ready.append((h, c))

            def flush(self):
                for (h, c) in self.ready:
                    self.on_final(self.fg[c], h, [self.acc[i, h, c][0] for i in self.prods])
                self.ready = []

            def run(self):
                self.flush()
                for t in list(self.todo):
                    self.term(t)
                    self.flush()

        def bias(k, h):
            return sh_ref[k, h * MH:(h + 1) * MH, :]

        for d in range(ND):
            st12, y0p, y3p = {}, {}, {}

            def fin12(X, h, v):
                st12[X, h] = ((v[0] + v[1]) + bias(1, h), a * (v[0] - v[1]) + bias(0, h))

            def fin34(X, h, v):
                p, q = st12[X, h]
                r, s = v[0] + v[1], b * (v[0] - v[1])
                o_ref[8 * d + 4 * X + 1, h * MH:(h + 1) * MH, :] = _silu2(q + s)
                o_ref[8 * d + 4 * X + 2, h * MH:(h + 1) * MH, :] = _silu2((a * a) * p + (b * b) * r)
                y0p[X, h] = p + r
                y3p[X, h] = (a * a) * q + (b * b) * s

            def fin_last(yp, off, kb):
                def f(X, h, v):
                    slab = 8 * d + 4 * X + off
                    o_ref[slab, h * MH:(h + 1) * MH, :] = _silu2(yp[X, h] + (v[0] + bias(kb, h)))
                    if d == ND - 1 and (slab, h) not in LATE:
                        out_half(step, slab, h).start()
                return f

            g12 = Group(d, (1, 2), 0, SEQ_12, fin12)
            g34 = Group(d, (3, 4), 1, SEQ_34, fin34)
            g0 = Group(d, (0,), 2, SEQ_0, fin_last(y0p, 0, 2))
            g5 = Group(d, (5,), 3, SEQ_5, fin_last(y3p, 3, 3))
            if first and d == 0:
                for grp in (g12, g34, g5):
                    for t in ((5, 3) if grp.fg[0] else (2, 4)):
                        grp.term(t)
                g0.rhs(2, 0)
                g0.rhs(4, 0)
                wrem_copy.wait()
                fcs[1].wait()
                remainder_lhs()
                g0.term(2)
                g0.term(4)
            g12.run()
            if first and d < 2:
                t = [t for t in g34.todo if t < 10][0]
                g34.todo.remove(t)
                g34.todo.insert(0, t)
                g34.rhs(t, 0)
                g34.rhs(t, 1)
                fcs[2 + d].wait()
            g34.run()
            if d == ND - 1:
                out_copy(step, 8 * d + 1, 2).start()
                out_copy(step, 8 * d + 5, 2).start()
            g5.run()
            g0.run()
            if d < ND - 1:
                out_copy(step, 8 * d, 8).start()

    def scoped_block(step):
        pl.run_scoped(lambda s_ref: block(step, s_ref), pltpu.VMEM((48, KH, TB), bf16))

    scoped_block(0)

    def body(step, carry):
        in_copy(step).wait()

        @pl.when(step >= 2)
        def _():
            out_wait_all(_sl(step))

        for slab, h in LATE:
            out_half(step - 1, slab, h).start()

        @pl.when(step + 1 < NS)
        def _():
            in_copy(step + 1).start()

        scoped_block(step)
        return carry

    jax.lax.fori_loop(1, NS, body, 0)
    for slab, h in LATE:
        out_half(NS - 1, slab, h).start()
    out_wait_all(NS % 2)
    out_wait_all((NS - 1) % 2)


@jax.jit
def pallas_standalone__batchnorm__sampling_kernel(
    x: jax.Array,
    w: jax.Array,
    mean: jax.Array,
    var: jax.Array,
    g: jax.Array,
    b: jax.Array,
):
    B, S, C = x.shape
    xt = jnp.transpose(x, (1, 2, 0))
    out = pl.pallas_call(
        _kernel,
        in_specs=[pl.BlockSpec(memory_space=pl.ANY)] * 6,
        out_specs=pl.BlockSpec(memory_space=pl.ANY),
        out_shape=jax.ShapeDtypeStruct((S, C, B), x.dtype),
        scratch_shapes=[pltpu.VMEM((3, C, C), bf16)] + [pltpu.VMEM((C,), bf16)] * 4 + [
            pltpu.VMEM((6, 7, 2, C // 2, 128), bf16),
            pltpu.VMEM((5, C, 128), bf16),
            pltpu.VMEM((4, C, 128), f32),
            pltpu.VMEM((4, C, 128), f32),
            pltpu.VMEM((2, S, C, TB), bf16),
            pltpu.VMEM((2, S, C, TB), bf16),
            pltpu.SMEM((4,), jnp.int32),
            pltpu.SemaphoreType.DMA((NSEM,)),
        ],
        compiler_params=pltpu.CompilerParams(
            vmem_limit_bytes=100 * 1024 * 1024,
            disable_bounds_checks=True,
            disable_semaphore_checks=True,
        ),
    )(xt, w, mean, var, g, b)
    return jnp.transpose(out, (2, 0, 1))
```

```python
import jax
import jax.numpy as jnp
import jax.experimental.pallas as pl
import jax.experimental.pallas.tpu as pltpu

f32 = jnp.float32
bf16 = jnp.bfloat16
u32 = jnp.uint32

A = 0.6875
Bp = 1.0 / A
TB = 128
KM = 512
KH = KM // 2
RS = 96
SWAP = (0, 1, 1, 0, 0, 1)
SDEF = {1: ((1, 1, 1), (2, 2, 1)), 2: ((1, 1, 1),), 3: ((1, 2, 1), (2, 2, -1)),
        4: ((2, 1, 1), (1, 1, -1)), 5: ((2, 2, 1),), 6: ((1, 1, 1), (1, 2, 1)),
        7: ((2, 1, 1), (2, 2, 1))}
USE = {1: ((0, 0, 1), (1, 1, 1)), 2: ((1, 0, 1), (1, 1, -1)), 3: ((0, 1, 1), (1, 1, 1)),
       4: ((0, 0, 1), (1, 0, 1)), 5: ((0, 0, -1), (0, 1, 1)), 6: ((1, 1, 1),), 7: ((0, 0, 1),),
       11: ((0, 0, 1),), 21: ((1, 0, 1),), 12: ((0, 1, 1),), 22: ((1, 1, 1),)}
SEQ_12 = (2, 4, 21, 12, 5, 3, 22, 11, 1, 6, 7)
SEQ_34 = (2, 4, 21, 12, 5, 3, 1, 22, 11, 6, 7)
SEQ_5 = (2, 4, 5, 3, 1, 6, 7)
WPOS = (2, 0, 2, 0)
SEQ_0 = (2, 4, 5, 3, 1, 6, 7)
FIRST = ((0, 5), (5, 9), (9, 17), (17, 32))
LATE = ((28, 1), (24, 0))
FIVE_FIRST = True
PS, WS, FS = 0, 4, 9
IS = FS + len(FIRST)
OS = IS + 2
NSEM = OS + 2


def _upk(v):
    return pltpu.bitcast(v, bf16)


def _dsm(lo, n):
    return pl.ds(lo if isinstance(lo, int) else pl.multiple_of(lo, n), n)


def _sl(st):
    return st % 2 if isinstance(st, int) else st & 1


def _silu2(h):
    return (h + h * jnp.tanh(h)).astype(bf16)


def _dot(l, r):
    return jnp.dot(_upk(l), r, preferred_element_type=f32)


def _kernel(x_hbm, w_hbm, m_hbm, v_hbm, g_hbm, b_hbm, o_hbm,
            wbuf, pm, pv, pg, pb, a_ref, r_ref, sc_ref, sh_ref, xbuf, obuf, z_ref, sem):
    S, C, B = x_hbm.shape
    ND = S // 8
    NS = B // TB
    MH = C // 2
    KR = C - KM
    a, b = A, Bp
    cc = a * a + b * b
    D = 1.0 / (2 * (b * b - a * a))
    a32, r32 = a_ref.bitcast(u32), r_ref.bitcast(u32)

    def x_copy(st, lo, hi, s):
        return pltpu.make_async_copy(
            x_hbm.at[pl.ds(lo, hi - lo), :, _dsm(st * TB, TB)],
            xbuf.at[_sl(st), pl.ds(lo, hi - lo)], s)

    def in_copy(st):
        return x_copy(st, 0, S, sem.at[IS + _sl(st)])

    def out_copy(st, lo, n):
        return pltpu.make_async_copy(
            obuf.at[_sl(st), pl.ds(lo, n)],
            o_hbm.at[pl.ds(lo, n), :, _dsm(st * TB, TB)], sem.at[OS + _sl(st)])

    def out_half(st, slab, h):
        return pltpu.make_async_copy(
            obuf.at[_sl(st), slab, pl.ds(h * MH, MH)],
            o_hbm.at[slab, pl.ds(h * MH, MH), _dsm(st * TB, TB)], sem.at[OS + _sl(st)])

    def out_wait_all(sl):
        pltpu.make_async_copy(obuf.at[sl], obuf.at[sl], sem.at[OS + sl]).wait()

    pcs = [pltpu.make_async_copy(s, d, sem.at[PS + i])
           for i, (s, d) in enumerate(((m_hbm, pm), (v_hbm, pv), (g_hbm, pg), (b_hbm, pb)))]

    def w_copy(r):
        return pltpu.make_async_copy(w_hbm.at[:, _dsm(r * 128, 128), :],
                                     wbuf.at[:, _dsm(r * 128, 128), :], sem.at[WS + r])

    wrem_copy = pltpu.make_async_copy(w_hbm.at[:, pl.ds(KM, KR), :],
                                      wbuf.at[:, pl.ds(KM, KR), :], sem.at[WS + 4])
    fcs = [x_copy(0, lo, hi, sem.at[FS + k]) for k, (lo, hi) in enumerate(FIRST)]

    def u_vals(gs, lo, n):
        sc = [sc_ref[k, lo:lo + n, :] for k in range(4)]
        u0 = gs[0] * sc[0]
        u5 = gs[2] * sc[1]
        e = D * u5
        ea = (b * b * D) * u0 - e
        eb = e - (a * a * D) * u0
        hb = gs[1] * sc[2]
        ha = gs[1] * sc[3]
        return [u0, ea - hb, ea + hb, eb + ha, eb - ha, u5]

    eye = (jax.lax.broadcasted_iota(jnp.int32, (128, 128), 0)
           == jax.lax.broadcasted_iota(jnp.int32, (128, 128), 1)).astype(f32).astype(bf16)

    def tr_rows(k, q, lo, n):
        out = []
        while n > 0:
            t, o = lo // 128, lo % 128
            m = min(n, 128 - o)
            wd = min(128, C - 128 * t)
            w = wbuf[k, _dsm(q * 128, 128), 128 * t:128 * t + wd]
            out.append(jax.lax.dot_general(eye[o:o + m, :wd], w, (((1,), (1,)), ((), ())),
                                           preferred_element_type=f32))
            lo, n = lo + m, n - m
        return out[0] if len(out) == 1 else jnp.concatenate(out, axis=0)

    def strassen_lhs(r, carry):
        z_ref[r] = 0
        z_ref[r + 2] = 0
        w_copy(r).wait()
        w_copy(r + 2).wait()
        for c in range(MH // RS):
            us = {}
            for h in range(2):
                lo = h * MH + c * RS
                gs = [[tr_rows(k, r + 2 * q, lo, RS) for k in range(3)] for q in range(2)]
                for q in range(2):
                    us[h, q] = u_vals(gs[q], lo, RS)
            for i in range(6):
                a11, a12, a21, a22 = us[0, 0][i], us[0, 1][i], us[1, 0][i], us[1, 1][i]
                for s, v in enumerate((a11 + a22, a21 + a22, a11, a22,
                                       a11 + a12, a21 - a11, a12 - a22)):
                    a_ref[i, s, r, c * RS:(c + 1) * RS, :] = v.astype(bf16)
        return carry

    def remainder_lhs():
        wr = [wbuf[k, KM:, :] for k in range(3)]
        us = u_vals([jnp.concatenate([w, w], axis=0).T.astype(f32) for w in wr], 0, C)
        low = jax.lax.broadcasted_iota(jnp.int32, (C, 2 * KR), 1) < KR
        for i in range(1, 5):
            r_ref[2 * i - 2] = jnp.where(low, us[i], us[0]).astype(bf16)
            r_ref[2 * i - 1] = jnp.where(low, us[i], us[5]).astype(bf16)
        r_ref[8] = jnp.where(low, us[5], us[0]).astype(bf16)

    for c in pcs + [w_copy(r) for r in (0, 2, 1, 3)] + [fcs[0], wrem_copy] + fcs[1:]:
        c.start()
    in_copy(1).start()
    for c in pcs:
        c.wait()
    mean, var, g, bb = (r[...].reshape(1, C).astype(f32) for r in (pm, pv, pg, pb))
    sc_all = 0.5 * g / jnp.sqrt(var + 1e-5)
    scc = jnp.broadcast_to(sc_all, (128, C)).T
    sc_ref[0] = -scc
    sc_ref[1] = scc
    sc_ref[2] = (b * D) * scc
    sc_ref[3] = (a * D) * scc
    sh = jnp.broadcast_to(0.5 * bb - mean * sc_all, (128, C)).T
    sh_ref[0] = sh
    sh_ref[1] = (b * b) * sh
    sh_ref[2] = (1.0 - b * b) * sh
    sh_ref[3] = (1.0 - a * a) * sh
    jax.lax.fori_loop(0, 2, strassen_lhs, 0)
    fcs[0].wait()

    def block(step, s_ref):
        first = isinstance(step, int)
        o_ref = obuf.at[_sl(step)]
        s32 = s_ref.bitcast(u32)

        def t_rows(j, lo, n, grp, cell):
            xb = xbuf.at[(step + z_ref[cell]) & 1]

            def dd(k):
                i = 4 * j - 1 + k
                return xb[i, lo:lo + n, :].astype(f32) if 0 <= i < S else None

            if grp == (1, 2):
                p = dd(4) - (b * b) * dd(2)
                q = a * dd(3) - b * dd(1)
                return p + q, p - q
            if grp == (3, 4):
                p = dd(4) - (a * a) * dd(2)
                q = b * dd(3) - a * dd(1)
                return p + q, p - q
            if grp == (0,):
                d0 = dd(0)
                return (cc * dd(2) - (dd(4) if d0 is None else dd(4) + d0),)
            d5 = dd(5)
            return ((dd(1) if d5 is None else dd(1) + d5) - cc * dd(3),)

        def to_bf16(v, e, lo):
            n = v.shape[0]
            s_ref[e, lo:lo + n, :] = v.astype(bf16)
            return _upk(s32[e, lo // 2:(lo + n) // 2, :])

        class Group:
            def __init__(self, d, prods, cell, seq, on_final):
                self.d, self.prods, self.cell, self.on_final = d, prods, cell, on_final
                self.fg = (1, 0) if SWAP[prods[0]] else (0, 1)
                self.todo = list(seq)
                self.blocks, self.rems, self.rhss = {}, {}, {}
                self.acc, self.left, self.ready = {}, {}, []
                for t in seq:
                    for (h, c, _) in USE[t]:
                        self.left[h, c] = self.left.get((h, c), 0) + 1

            def blk(self, k, c):
                if (k, c) not in self.blocks:
                    self.blocks[k, c] = t_rows(2 * self.d + self.fg[c - 1], (k - 1) * KH, KH,
                                               self.prods, self.cell)
                return self.blocks[k, c]

            def rem(self, X):
                if X not in self.rems:
                    ts = t_rows(2 * self.d + X, KM, KR, self.prods, self.cell)
                    tl, tr = (t_rows(2 * self.d + k, KM, KR, (5,) if X else (0,), self.cell)[0]
                              for k in range(2))
                    ce, lo = (b * b * D, -b * D) if self.prods == (1, 2) else (-a * a * D, a * D)
                    if X == 0:
                        e, o = ce * tl, lo * tr
                        zs = (e - o, e + o)
                    else:
                        e, o = (-ce) * tl, lo * tr
                        zs = (e + o, e - o)
                    self.rems[X] = [to_bf16(jnp.concatenate([t, z], axis=0), 8 * i + 7, 2 * KR * X)
                                    for i, t, z in zip(self.prods, ts, zs)]
                return self.rems[X]

            def rhs(self, t, n):
                if (t, n) not in self.rhss:
                    vs = [self.blk(k, c)[n] for (k, c, _) in SDEF[t]]
                    if len(vs) == 2:
                        vs = [vs[0] + vs[1] if SDEF[t][1][2] > 0 else vs[0] - vs[1]]
                    self.rhss[t, n] = to_bf16(vs[0], 8 * self.prods[n] + t - 1, 0)
                return self.rhss[t, n]

            def term(self, t):
                self.todo.remove(t)
                for n, i in enumerate(self.prods):
                    if t < 10:
                        l = jnp.concatenate([a32[i, t - 1, 0], a32[i, t - 1, 1]], axis=1)
                        v = _dot(l, self.rhs(t, n))
                    else:
                        h, X = t // 10 - 1, self.fg[t % 10 - 1]
                        v = _dot(r32[2 * i - 2 + X, h * MH // 2:(h + 1) * MH // 2, :], self.rem(X)[n])
                    for (h, c, sg) in USE[t]:
                        k = (i, h, c)
                        if k not in self.acc:
                            self.acc[k] = (v, sg)
                        else:
                            p, ps = self.acc[k]
                            self.acc[k] = ((p + v, sg) if ps == sg
                                           else (p - v if ps > 0 else v - p, 1))
                for (h, c, _) in USE[t]:
                    self.left[h, c] -= 1
                    if self.left[h, c] == 0:
                        self.ready.append((h, c))

            def flush(self):
                for (h, c) in self.ready:
                    self.on_final(self.fg[c], h, [self.acc[i, h, c][0] for i in self.prods])
                self.ready = []

            def run(self):
                self.flush()
                for t in list(self.todo):
                    self.term(t)
                    self.flush()

        def bias(k, h):
            return sh_ref[k, h * MH:(h + 1) * MH, :]

        for d in range(ND):
            st12, y0p, y3p = {}, {}, {}

            def fin12(X, h, v):
                st12[X, h] = ((v[0] + v[1]) + bias(1, h), a * (v[0] - v[1]) + bias(0, h))

            def fin34(X, h, v):
                p, q = st12[X, h]
                r, s = v[0] + v[1], b * (v[0] - v[1])
                o_ref[8 * d + 4 * X + 1, h * MH:(h + 1) * MH, :] = _silu2(q + s)
                o_ref[8 * d + 4 * X + 2, h * MH:(h + 1) * MH, :] = _silu2((a * a) * p + (b * b) * r)
                y0p[X, h] = p + r
                y3p[X, h] = (a * a) * q + (b * b) * s

            def fin_last(yp, off, kb):
                def f(X, h, v):
                    slab = 8 * d + 4 * X + off
                    y = yp[X, h] + (v[0] + bias(kb, h))
                    if (off == 3) == (X == 0):
                        y = y + shared[h]
                    o_ref[slab, h * MH:(h + 1) * MH, :] = _silu2(y)
                    if d == ND - 1 and (slab, h) not in LATE:
                        out_half(step, slab, h).start()
                return f

            shared = []

            def shared_tile(pos):
                if pos == WPOS[d] and not shared:
                    t = jnp.concatenate([t_rows(2 * d, KM, KR, (5,), 3)[0],
                                         t_rows(2 * d + 1, KM, KR, (0,), 3)[0]], axis=0)
                    t = to_bf16(t, 7, 0)
                    for h in range(2):
                        shared.append(_dot(r32[8, h * MH // 2:(h + 1) * MH // 2, :], t))

            g12 = Group(d, (1, 2), 0, SEQ_12, fin12)
            g34 = Group(d, (3, 4), 1, SEQ_34, fin34)
            g0 = Group(d, (0,), 2, SEQ_0, fin_last(y0p, 0, 2))
            g5 = Group(d, (5,), 3, SEQ_5, fin_last(y3p, 3, 3))
            if first and d == 0:
                for grp in (g12, g34, g5):
                    for t in ((5, 3) if grp.fg[0] else (2, 4)):
                        grp.term(t)
                g0.rhs(2, 0)
                g0.rhs(4, 0)
                wrem_copy.wait()
                fcs[1].wait()
                remainder_lhs()
                g0.term(2)
                g0.term(4)
            shared_tile(0)
            g12.run()
            if first and d < 2:
                t = [t for t in g34.todo if t < 10][0]
                g34.todo.remove(t)
                g34.todo.insert(0, t)
                g34.rhs(t, 0)
                g34.rhs(t, 1)
                fcs[2 + d].wait()
            shared_tile(1)
            g34.run()
            if d == ND - 1:
                out_copy(step, 8 * d + 1, 2).start()
                out_copy(step, 8 * d + 5, 2).start()
            shared_tile(2)
            for grp in ((g5, g0) if FIVE_FIRST else (g0, g5)):
                grp.run()
            if d < ND - 1:
                out_copy(step, 8 * d, 8).start()

    def scoped_block(step):
        pl.run_scoped(lambda s_ref: block(step, s_ref), pltpu.VMEM((48, KH, TB), bf16))

    scoped_block(0)

    def body(step, carry):
        in_copy(step).wait()

        @pl.when(step >= 2)
        def _():
            out_wait_all(_sl(step))

        for slab, h in LATE:
            out_half(step - 1, slab, h).start()

        @pl.when(step + 1 < NS)
        def _():
            in_copy(step + 1).start()

        scoped_block(step)
        return carry

    jax.lax.fori_loop(1, NS, body, 0)
    for slab, h in LATE:
        out_half(NS - 1, slab, h).start()
    out_wait_all(NS % 2)
    out_wait_all((NS - 1) % 2)


@jax.jit
def pallas_standalone__batchnorm__sampling_kernel(
    x: jax.Array,
    w: jax.Array,
    mean: jax.Array,
    var: jax.Array,
    g: jax.Array,
    b: jax.Array,
):
    B, S, C = x.shape
    xt = jnp.transpose(x, (1, 2, 0))
    out = pl.pallas_call(
        _kernel,
        in_specs=[pl.BlockSpec(memory_space=pl.ANY)] * 6,
        out_specs=pl.BlockSpec(memory_space=pl.ANY),
        out_shape=jax.ShapeDtypeStruct((S, C, B), x.dtype),
        scratch_shapes=[pltpu.VMEM((3, C, C), bf16)] + [pltpu.VMEM((C,), bf16)] * 4 + [
            pltpu.VMEM((6, 7, 2, C // 2, 128), bf16),
            pltpu.VMEM((9, C, 128), bf16),
            pltpu.VMEM((4, C, 128), f32),
            pltpu.VMEM((4, C, 128), f32),
            pltpu.VMEM((2, S, C, TB), bf16),
            pltpu.VMEM((2, S, C, TB), bf16),
            pltpu.SMEM((4,), jnp.int32),
            pltpu.SemaphoreType.DMA((NSEM,)),
        ],
        compiler_params=pltpu.CompilerParams(
            vmem_limit_bytes=100 * 1024 * 1024,
            disable_bounds_checks=True,
            disable_semaphore_checks=True,
        ),
    )(xt, w, mean, var, g, b)
    return jnp.transpose(out, (2, 0, 1))
```

```python
import jax
import jax.numpy as jnp
import jax.experimental.pallas as pl
import jax.experimental.pallas.tpu as pltpu

f32 = jnp.float32
bf16 = jnp.bfloat16
u32 = jnp.uint32

A = 0.6875
Bp = 1.0 / A
TB = 128
KM = 512
KH = KM // 2
RS = 96
SWAP = (0, 1, 1, 0, 0, 1)
SDEF = {1: ((1, 1, 1), (2, 2, 1)), 2: ((1, 1, 1),), 3: ((1, 2, 1), (2, 2, -1)),
        4: ((2, 1, 1), (1, 1, -1)), 5: ((2, 2, 1),), 6: ((1, 1, 1), (1, 2, 1)),
        7: ((2, 1, 1), (2, 2, 1))}
USE = {1: ((0, 0, 1), (1, 1, 1)), 2: ((1, 0, 1), (1, 1, -1)), 3: ((0, 1, 1), (1, 1, 1)),
       4: ((0, 0, 1), (1, 0, 1)), 5: ((0, 0, -1), (0, 1, 1)), 6: ((1, 1, 1),), 7: ((0, 0, 1),),
       11: ((0, 0, 1),), 21: ((1, 0, 1),), 12: ((0, 1, 1),), 22: ((1, 1, 1),)}
SEQ_12 = (2, 4, 21, 12, 5, 3, 22, 11, 1, 6, 7)
SEQ_34 = (2, 4, 21, 12, 5, 3, 1, 22, 11, 6, 7)
SEQ_05 = (2, 4, 5, 3, 1, 6, 7)
FIRST = ((0, 5), (5, 9), (9, 17), (17, 32))
LATE = ((28, 1), (24, 0))
PS, WS, FS = 0, 4, 9
IS = FS + len(FIRST)
OS = IS + 2
NSEM = OS + 2


def _upk(v):
    return pltpu.bitcast(v, bf16)


def _dsm(lo, n):
    return pl.ds(lo if isinstance(lo, int) else pl.multiple_of(lo, n), n)


def _sl(st):
    return st % 2 if isinstance(st, int) else st & 1


def _silu2(h):
    return (h + h * jnp.tanh(h)).astype(bf16)


def _dot(l, r):
    return jnp.dot(_upk(l), r, preferred_element_type=f32)


def _kernel(x_hbm, w_hbm, m_hbm, v_hbm, g_hbm, b_hbm, o_hbm,
            wbuf, pm, pv, pg, pb, a_ref, r_ref, sc_ref, sh_ref, xbuf, obuf, z_ref, sem):
    S, C, B = x_hbm.shape
    ND = S // 8
    NS = B // TB
    MH = C // 2
    KR = C - KM
    a, b = A, Bp
    cc = a * a + b * b
    D = 1.0 / (2 * (b * b - a * a))
    a32, r32 = a_ref.bitcast(u32), r_ref.bitcast(u32)

    def x_copy(st, lo, hi, s):
        return pltpu.make_async_copy(
            x_hbm.at[pl.ds(lo, hi - lo), :, _dsm(st * TB, TB)],
            xbuf.at[_sl(st), pl.ds(lo, hi - lo)], s)

    def in_copy(st):
        return x_copy(st, 0, S, sem.at[IS + _sl(st)])

    def out_copy(st, lo, n):
        return pltpu.make_async_copy(
            obuf.at[_sl(st), pl.ds(lo, n)],
            o_hbm.at[pl.ds(lo, n), :, _dsm(st * TB, TB)], sem.at[OS + _sl(st)])

    def out_half(st, slab, h):
        return pltpu.make_async_copy(
            obuf.at[_sl(st), slab, pl.ds(h * MH, MH)],
            o_hbm.at[slab, pl.ds(h * MH, MH), _dsm(st * TB, TB)], sem.at[OS + _sl(st)])

    def out_wait_all(sl):
        pltpu.make_async_copy(obuf.at[sl], obuf.at[sl], sem.at[OS + sl]).wait()

    pcs = [pltpu.make_async_copy(s, d, sem.at[PS + i])
           for i, (s, d) in enumerate(((m_hbm, pm), (v_hbm, pv), (g_hbm, pg), (b_hbm, pb)))]

    def w_copy(r):
        return pltpu.make_async_copy(w_hbm.at[:, _dsm(r * 128, 128), :],
                                     wbuf.at[:, _dsm(r * 128, 128), :], sem.at[WS + r])

    wrem_copy = pltpu.make_async_copy(w_hbm.at[:, pl.ds(KM, KR), :],
                                      wbuf.at[:, pl.ds(KM, KR), :], sem.at[WS + 4])
    fcs = [x_copy(0, lo, hi, sem.at[FS + k]) for k, (lo, hi) in enumerate(FIRST)]

    def u_vals(gs, lo, n):
        sc = [sc_ref[k, lo:lo + n, :] for k in range(4)]
        u0 = gs[0] * sc[0]
        u5 = gs[2] * sc[1]
        e = D * u5
        ea = (b * b * D) * u0 - e
        eb = e - (a * a * D) * u0
        hb = gs[1] * sc[2]
        ha = gs[1] * sc[3]
        return [u0, ea - hb, ea + hb, eb + ha, eb - ha, u5]

    eye = (jax.lax.broadcasted_iota(jnp.int32, (128, 128), 0)
           == jax.lax.broadcasted_iota(jnp.int32, (128, 128), 1)).astype(f32).astype(bf16)

    def tr_rows(k, q, lo, n):
        out = []
        while n > 0:
            t, o = lo // 128, lo % 128
            m = min(n, 128 - o)
            wd = min(128, C - 128 * t)
            w = wbuf[k, _dsm(q * 128, 128), 128 * t:128 * t + wd]
            out.append(jax.lax.dot_general(eye[o:o + m, :wd], w, (((1,), (1,)), ((), ())),
                                           preferred_element_type=f32))
            lo, n = lo + m, n - m
        return out[0] if len(out) == 1 else jnp.concatenate(out, axis=0)

    def strassen_lhs(r, carry):
        z_ref[r] = 0
        z_ref[r + 2] = 0
        w_copy(r).wait()
        w_copy(r + 2).wait()
        for c in range(MH // RS):
            us = {}
            for h in range(2):
                lo = h * MH + c * RS
                gs = [[tr_rows(k, r + 2 * q, lo, RS) for k in range(3)] for q in range(2)]
                for q in range(2):
                    us[h, q] = u_vals(gs[q], lo, RS)
            for i in range(6):
                a11, a12, a21, a22 = us[0, 0][i], us[0, 1][i], us[1, 0][i], us[1, 1][i]
                for s, v in enumerate((a11 + a22, a21 + a22, a11, a22,
                                       a11 + a12, a21 - a11, a12 - a22)):
                    a_ref[i, s, r, c * RS:(c + 1) * RS, :] = v.astype(bf16)
        return carry

    def remainder_lhs():
        wr = [wbuf[k, KM:, :] for k in range(3)]
        us = u_vals([jnp.concatenate([w, w], axis=0).T.astype(f32) for w in wr], 0, C)
        low = jax.lax.broadcasted_iota(jnp.int32, (C, 2 * KR), 1) < KR
        for i in range(1, 5):
            r_ref[2 * i - 2] = jnp.where(low, us[i], us[0]).astype(bf16)
            r_ref[2 * i - 1] = jnp.where(low, us[i], us[5]).astype(bf16)
        r_ref[8] = jnp.where(low, us[5], us[0]).astype(bf16)

    for c in pcs + [w_copy(r) for r in (0, 2, 1, 3)] + [fcs[0], wrem_copy] + fcs[1:]:
        c.start()
    in_copy(1).start()
    for c in pcs:
        c.wait()
    mean, var, g, bb = (r[...].reshape(1, C).astype(f32) for r in (pm, pv, pg, pb))
    sc_all = 0.5 * g / jnp.sqrt(var + 1e-5)
    scc = jnp.broadcast_to(sc_all, (128, C)).T
    sc_ref[0] = -scc
    sc_ref[1] = scc
    sc_ref[2] = (b * D) * scc
    sc_ref[3] = (a * D) * scc
    sh = jnp.broadcast_to(0.5 * bb - mean * sc_all, (128, C)).T
    sh_ref[0] = sh
    sh_ref[1] = (b * b) * sh
    sh_ref[2] = (1.0 - b * b) * sh
    sh_ref[3] = (1.0 - a * a) * sh
    jax.lax.fori_loop(0, 2, strassen_lhs, 0)
    fcs[0].wait()

    def block(step, s_ref):
        first = isinstance(step, int)
        o_ref = obuf.at[_sl(step)]
        s32 = s_ref.bitcast(u32)

        def t_rows(j, lo, n, grp, cell):
            xb = xbuf.at[(step + z_ref[cell]) & 1]

            def dd(k):
                i = 4 * j - 1 + k
                return xb[i, lo:lo + n, :].astype(f32) if 0 <= i < S else None

            if grp == (1, 2):
                p = dd(4) - (b * b) * dd(2)
                q = a * dd(3) - b * dd(1)
                return p + q, p - q
            if grp == (3, 4):
                p = dd(4) - (a * a) * dd(2)
                q = b * dd(3) - a * dd(1)
                return p + q, p - q
            if grp == (0,):
                d0 = dd(0)
                return (cc * dd(2) - (dd(4) if d0 is None else dd(4) + d0),)
            d5 = dd(5)
            return ((dd(1) if d5 is None else dd(1) + d5) - cc * dd(3),)

        def to_bf16(v, e, lo):
            n = v.shape[0]
            s_ref[e, lo:lo + n, :] = v.astype(bf16)
            return _upk(s32[e, lo // 2:(lo + n) // 2, :])

        class Group:
            def __init__(self, d, prods, cell, seq, on_final):
                self.d, self.prods, self.cell, self.on_final = d, prods, cell, on_final
                self.fg = (1, 0) if SWAP[prods[0]] else (0, 1)
                self.todo = list(seq)
                self.blocks, self.rems, self.rhss = {}, {}, {}
                self.acc, self.left, self.ready = {}, {}, []
                for t in seq:
                    for (h, c, _) in USE[t]:
                        self.left[h, c] = self.left.get((h, c), 0) + 1

            def blk(self, k, c):
                if (k, c) not in self.blocks:
                    self.blocks[k, c] = t_rows(2 * self.d + self.fg[c - 1], (k - 1) * KH, KH,
                                               self.prods, self.cell)
                return self.blocks[k, c]

            def rem(self, X):
                if X not in self.rems:
                    ts = t_rows(2 * self.d + X, KM, KR, self.prods, self.cell)
                    tl, tr = (t_rows(2 * self.d + k, KM, KR, (5,) if X else (0,), self.cell)[0]
                              for k in range(2))
                    ce, lo = (b * b * D, -b * D) if self.prods == (1, 2) else (-a * a * D, a * D)
                    if X == 0:
                        e, o = ce * tl, lo * tr
                        zs = (e - o, e + o)
                    else:
                        e, o = (-ce) * tl, lo * tr
                        zs = (e + o, e - o)
                    self.rems[X] = [to_bf16(jnp.concatenate([t, z], axis=0), 8 * i + 7, 2 * KR * X)
                                    for i, t, z in zip(self.prods, ts, zs)]
                return self.rems[X]

            def rhs(self, t, n):
                if (t, n) not in self.rhss:
                    vs = [self.blk(k, c)[n] for (k, c, _) in SDEF[t]]
                    if len(vs) == 2:
                        vs = [vs[0] + vs[1] if SDEF[t][1][2] > 0 else vs[0] - vs[1]]
                    self.rhss[t, n] = to_bf16(vs[0], 8 * self.prods[n] + t - 1, 0)
                return self.rhss[t, n]

            def term(self, t):
                self.todo.remove(t)
                for n, i in enumerate(self.prods):
                    if t < 10:
                        l = jnp.concatenate([a32[i, t - 1, 0], a32[i, t - 1, 1]], axis=1)
                        v = _dot(l, self.rhs(t, n))
                    else:
                        h, X = t // 10 - 1, self.fg[t % 10 - 1]
                        v = _dot(r32[2 * i - 2 + X, h * MH // 2:(h + 1) * MH // 2, :], self.rem(X)[n])
                    for (h, c, sg) in USE[t]:
                        k = (i, h, c)
                        if k not in self.acc:
                            self.acc[k] = (v, sg)
                        else:
                            p, ps = self.acc[k]
                            self.acc[k] = ((p + v, sg) if ps == sg
                                           else (p - v if ps > 0 else v - p, 1))
                for (h, c, _) in USE[t]:
                    self.left[h, c] -= 1
                    if self.left[h, c] == 0:
                        self.ready.append((h, c))

            def flush(self):
                for (h, c) in self.ready:
                    self.on_final(self.fg[c], h, [self.acc[i, h, c][0] for i in self.prods])
                self.ready = []

            def run(self):
                self.flush()
                for t in list(self.todo):
                    self.term(t)
                    self.flush()

        def bias(k, h):
            return sh_ref[k, h * MH:(h + 1) * MH, :]

        for d in range(ND):
            st12, y0p, y3p = {}, {}, {}

            def fin12(X, h, v):
                st12[X, h] = ((v[0] + v[1]) + bias(1, h), a * (v[0] - v[1]) + bias(0, h))

            def fin34(X, h, v):
                p, q = st12[X, h]
                r, s = v[0] + v[1], b * (v[0] - v[1])
                o_ref[8 * d + 4 * X + 1, h * MH:(h + 1) * MH, :] = _silu2(q + s)
                o_ref[8 * d + 4 * X + 2, h * MH:(h + 1) * MH, :] = _silu2((a * a) * p + (b * b) * r)
                y0p[X, h] = p + r
                y3p[X, h] = (a * a) * q + (b * b) * s

            def fin_last(yp, off, kb):
                def f(X, h, v):
                    slab = 8 * d + 4 * X + off
                    y = yp[X, h] + (v[0] + bias(kb, h))
                    if (off == 3) == (X == 0):
                        y = y + shared[h]
                    o_ref[slab, h * MH:(h + 1) * MH, :] = _silu2(y)
                    if d == ND - 1 and (slab, h) not in LATE:
                        out_half(step, slab, h).start()
                return f

            shared = []

            def shared_tile():
                if not shared:
                    t = jnp.concatenate([t_rows(2 * d, KM, KR, (5,), 3)[0],
                                         t_rows(2 * d + 1, KM, KR, (0,), 3)[0]], axis=0)
                    t = to_bf16(t, 7, 0)
                    for h in range(2):
                        shared.append(_dot(r32[8, h * MH // 2:(h + 1) * MH // 2, :], t))

            g12 = Group(d, (1, 2), 0, SEQ_12, fin12)
            g34 = Group(d, (3, 4), 1, SEQ_34, fin34)
            g0 = Group(d, (0,), 2, SEQ_05, fin_last(y0p, 0, 2))
            g5 = Group(d, (5,), 3, SEQ_05, fin_last(y3p, 3, 3))
            if first and d == 0:
                for grp in (g12, g34, g5):
                    for t in ((5, 3) if grp.fg[0] else (2, 4)):
                        grp.term(t)
                g0.rhs(2, 0)
                g0.rhs(4, 0)
                wrem_copy.wait()
                fcs[1].wait()
                remainder_lhs()
                g0.term(2)
                g0.term(4)
            if d % 2:
                shared_tile()
            g12.run()
            if first and d < 2:
                t = [t for t in g34.todo if t < 10][0]
                g34.todo.remove(t)
                g34.todo.insert(0, t)
                g34.rhs(t, 0)
                g34.rhs(t, 1)
                fcs[2 + d].wait()
            g34.run()
            if d == ND - 1:
                out_copy(step, 8 * d + 1, 2).start()
                out_copy(step, 8 * d + 5, 2).start()
            shared_tile()
            g5.run()
            g0.run()
            if d < ND - 1:
                out_copy(step, 8 * d, 8).start()
            if d == 0 and not first:
                for slab, h in LATE:
                    out_half(step - 1, slab, h).start()

    def scoped_block(step):
        pl.run_scoped(lambda s_ref: block(step, s_ref), pltpu.VMEM((48, KH, TB), bf16))

    scoped_block(0)

    def body(step, carry):
        in_copy(step).wait()

        @pl.when(step >= 2)
        def _():
            out_wait_all(_sl(step))

        @pl.when(step + 1 < NS)
        def _():
            in_copy(step + 1).start()

        scoped_block(step)
        return carry

    jax.lax.fori_loop(1, NS, body, 0)
    for slab, h in LATE:
        out_half(NS - 1, slab, h).start()
    out_wait_all(NS % 2)
    out_wait_all((NS - 1) % 2)


@jax.jit
def pallas_standalone__batchnorm__sampling_kernel(
    x: jax.Array,
    w: jax.Array,
    mean: jax.Array,
    var: jax.Array,
    g: jax.Array,
    b: jax.Array,
):
    B, S, C = x.shape
    xt = jnp.transpose(x, (1, 2, 0))
    out = pl.pallas_call(
        _kernel,
        in_specs=[pl.BlockSpec(memory_space=pl.ANY)] * 6,
        out_specs=pl.BlockSpec(memory_space=pl.ANY),
        out_shape=jax.ShapeDtypeStruct((S, C, B), x.dtype),
        scratch_shapes=[pltpu.VMEM((3, C, C), bf16)] + [pltpu.VMEM((C,), bf16)] * 4 + [
            pltpu.VMEM((6, 7, 2, C // 2, 128), bf16),
            pltpu.VMEM((9, C, 128), bf16),
            pltpu.VMEM((4, C, 128), f32),
            pltpu.VMEM((4, C, 128), f32),
            pltpu.VMEM((2, S, C, TB), bf16),
            pltpu.VMEM((2, S, C, TB), bf16),
            pltpu.SMEM((4,), jnp.int32),
            pltpu.SemaphoreType.DMA((NSEM,)),
        ],
        compiler_params=pltpu.CompilerParams(
            vmem_limit_bytes=100 * 1024 * 1024,
            disable_bounds_checks=True,
            disable_semaphore_checks=True,
        ),
    )(xt, w, mean, var, g, b)
    return jnp.transpose(out, (2, 0, 1))
```

```python
import jax
import jax.numpy as jnp
import jax.experimental.pallas as pl
import jax.experimental.pallas.tpu as pltpu

f32 = jnp.float32
bf16 = jnp.bfloat16
u32 = jnp.uint32

A = 0.6875
Bp = 1.0 / A
TB = 128
KM = 512
KH = KM // 2
RS = 96
SWAP = (0, 1, 1, 0, 0, 1)
SDEF = {1: ((1, 1, 1), (2, 2, 1)), 2: ((1, 1, 1),), 3: ((1, 2, 1), (2, 2, -1)),
        4: ((2, 1, 1), (1, 1, -1)), 5: ((2, 2, 1),), 6: ((1, 1, 1), (1, 2, 1)),
        7: ((2, 1, 1), (2, 2, 1))}
USE = {1: ((0, 0, 1), (1, 1, 1)), 2: ((1, 0, 1), (1, 1, -1)), 3: ((0, 1, 1), (1, 1, 1)),
       4: ((0, 0, 1), (1, 0, 1)), 5: ((0, 0, -1), (0, 1, 1)), 6: ((1, 1, 1),), 7: ((0, 0, 1),),
       11: ((0, 0, 1),), 21: ((1, 0, 1),), 12: ((0, 1, 1),), 22: ((1, 1, 1),)}
SEQ_12 = (2, 4, 21, 12, 5, 3, 22, 11, 1, 6, 7)
SEQ_34 = (2, 4, 21, 12, 5, 3, 1, 22, 11, 6, 7)
SEQ_05 = (2, 4, 5, 3, 1, 6, 7)
FIRST = ((0, 5), (5, 9), (9, 17), (17, 32))
LATE = ((28, 1), (24, 0))
PS, WS, FS = 0, 4, 9
IS = FS + len(FIRST)
OS = IS + 2
NSEM = OS + 2


def _upk(v):
    return pltpu.bitcast(v, bf16)


def _dsm(lo, n):
    return pl.ds(lo if isinstance(lo, int) else pl.multiple_of(lo, n), n)


def _sl(st):
    return st % 2 if isinstance(st, int) else st & 1


def _silu2(h):
    return (h + h * jnp.tanh(h)).astype(bf16)


def _dot(l, r):
    return jnp.dot(_upk(l), r, preferred_element_type=f32)


def _kernel(x_hbm, w_hbm, m_hbm, v_hbm, g_hbm, b_hbm, o_hbm,
            wbuf, pm, pv, pg, pb, a_ref, r_ref, sc_ref, sh_ref, xbuf, obuf, z_ref, sem):
    S, C, B = x_hbm.shape
    ND = S // 8
    NS = B // TB
    MH = C // 2
    KR = C - KM
    a, b = A, Bp
    cc = a * a + b * b
    D = 1.0 / (2 * (b * b - a * a))
    a32, r32 = a_ref.bitcast(u32), r_ref.bitcast(u32)

    def x_copy(st, lo, hi, s):
        return pltpu.make_async_copy(
            x_hbm.at[pl.ds(lo, hi - lo), :, _dsm(st * TB, TB)],
            xbuf.at[_sl(st), pl.ds(lo, hi - lo)], s)

    def in_copy(st):
        return x_copy(st, 0, S, sem.at[IS + _sl(st)])

    def out_copy(st, lo, n):
        return pltpu.make_async_copy(
            obuf.at[_sl(st), pl.ds(lo, n)],
            o_hbm.at[pl.ds(lo, n), :, _dsm(st * TB, TB)], sem.at[OS + _sl(st)])

    def out_half(st, slab, h):
        return pltpu.make_async_copy(
            obuf.at[_sl(st), slab, pl.ds(h * MH, MH)],
            o_hbm.at[slab, pl.ds(h * MH, MH), _dsm(st * TB, TB)], sem.at[OS + _sl(st)])

    def out_wait_all(sl):
        pltpu.make_async_copy(obuf.at[sl], obuf.at[sl], sem.at[OS + sl]).wait()

    pcs = [pltpu.make_async_copy(s, d, sem.at[PS + i])
           for i, (s, d) in enumerate(((m_hbm, pm), (v_hbm, pv), (g_hbm, pg), (b_hbm, pb)))]

    def w_copy(r):
        return pltpu.make_async_copy(w_hbm.at[:, _dsm(r * 128, 128), :],
                                     wbuf.at[:, _dsm(r * 128, 128), :], sem.at[WS + r])

    wrem_copy = pltpu.make_async_copy(w_hbm.at[:, pl.ds(KM, KR), :],
                                      wbuf.at[:, pl.ds(KM, KR), :], sem.at[WS + 4])
    fcs = [x_copy(0, lo, hi, sem.at[FS + k]) for k, (lo, hi) in enumerate(FIRST)]

    def u_vals(gs, lo, n):
        sc = [sc_ref[k, lo:lo + n, :] for k in range(4)]
        u0 = gs[0] * sc[0]
        u5 = gs[2] * sc[1]
        e = D * u5
        ea = (b * b * D) * u0 - e
        eb = e - (a * a * D) * u0
        hb = gs[1] * sc[2]
        ha = gs[1] * sc[3]
        return [u0, ea - hb, ea + hb, eb + ha, eb - ha, u5]

    eye = (jax.lax.broadcasted_iota(jnp.int32, (128, 128), 0)
           == jax.lax.broadcasted_iota(jnp.int32, (128, 128), 1)).astype(f32).astype(bf16)

    def tr_rows(k, q, lo, n):
        out = []
        while n > 0:
            t, o = lo // 128, lo % 128
            m = min(n, 128 - o)
            wd = min(128, C - 128 * t)
            w = wbuf[k, _dsm(q * 128, 128), 128 * t:128 * t + wd]
            out.append(jax.lax.dot_general(eye[o:o + m, :wd], w, (((1,), (1,)), ((), ())),
                                           preferred_element_type=f32))
            lo, n = lo + m, n - m
        return out[0] if len(out) == 1 else jnp.concatenate(out, axis=0)

    def strassen_lhs(r, carry):
        z_ref[r] = 0
        z_ref[r + 2] = 0
        w_copy(r).wait()
        w_copy(r + 2).wait()
        for c in range(MH // RS):
            us = {}
            for h in range(2):
                lo = h * MH + c * RS
                gs = [[tr_rows(k, r + 2 * q, lo, RS) for k in range(3)] for q in range(2)]
                for q in range(2):
                    us[h, q] = u_vals(gs[q], lo, RS)
            for i in range(6):
                a11, a12, a21, a22 = us[0, 0][i], us[0, 1][i], us[1, 0][i], us[1, 1][i]
                for s, v in enumerate((a11 + a22, a21 + a22, a11, a22,
                                       a11 + a12, a21 - a11, a12 - a22)):
                    a_ref[i, s, r, c * RS:(c + 1) * RS, :] = v.astype(bf16)
        return carry

    def remainder_lhs():
        wr = [wbuf[k, KM:, :] for k in range(3)]
        us = u_vals([jnp.concatenate([w, w], axis=0).T.astype(f32) for w in wr], 0, C)
        low = jax.lax.broadcasted_iota(jnp.int32, (C, 2 * KR), 1) < KR
        for i in range(1, 5):
            r_ref[2 * i - 2] = jnp.where(low, us[i], us[0]).astype(bf16)
            r_ref[2 * i - 1] = jnp.where(low, us[i], us[5]).astype(bf16)
        r_ref[8] = jnp.where(low, us[5], us[0]).astype(bf16)

    for c in pcs + [w_copy(r) for r in (0, 2, 1, 3)] + [fcs[0], wrem_copy] + fcs[1:]:
        c.start()
    in_copy(1).start()
    for c in pcs:
        c.wait()
    mean, var, g, bb = (r[...].reshape(1, C).astype(f32) for r in (pm, pv, pg, pb))
    sc_all = 0.5 * g / jnp.sqrt(var + 1e-5)
    scc = jnp.broadcast_to(sc_all, (128, C)).T
    sc_ref[0] = -scc
    sc_ref[1] = scc
    sc_ref[2] = (b * D) * scc
    sc_ref[3] = (a * D) * scc
    sh = jnp.broadcast_to(0.5 * bb - mean * sc_all, (128, C)).T
    sh_ref[0] = sh
    sh_ref[1] = (b * b) * sh
    sh_ref[2] = (1.0 - b * b) * sh
    sh_ref[3] = (1.0 - a * a) * sh
    jax.lax.fori_loop(0, 2, strassen_lhs, 0)
    fcs[0].wait()

    def block(step, s_ref):
        first = isinstance(step, int)
        o_ref = obuf.at[_sl(step)]
        s32 = s_ref.bitcast(u32)

        def t_rows(j, lo, n, grp, cell):
            xb = xbuf.at[(step + z_ref[cell]) & 1]

            def dd(k):
                i = 4 * j - 1 + k
                return xb[i, lo:lo + n, :].astype(f32) if 0 <= i < S else None

            if grp == (1, 2):
                p = dd(4) - (b * b) * dd(2)
                q = a * dd(3) - b * dd(1)
                return p + q, p - q
            if grp == (3, 4):
                p = dd(4) - (a * a) * dd(2)
                q = b * dd(3) - a * dd(1)
                return p + q, p - q
            if grp == (0,):
                d0 = dd(0)
                return (cc * dd(2) - (dd(4) if d0 is None else dd(4) + d0),)
            d5 = dd(5)
            return ((dd(1) if d5 is None else dd(1) + d5) - cc * dd(3),)

        def to_bf16(v, e, lo):
            n = v.shape[0]
            s_ref[e, lo:lo + n, :] = v.astype(bf16)
            return _upk(s32[e, lo // 2:(lo + n) // 2, :])

        class Group:
            def __init__(self, d, prods, cell, seq, on_final):
                self.d, self.prods, self.cell, self.on_final = d, prods, cell, on_final
                self.fg = (1, 0) if SWAP[prods[0]] else (0, 1)
                self.todo = list(seq)
                self.blocks, self.rems, self.rhss = {}, {}, {}
                self.acc, self.left, self.ready = {}, {}, []
                for t in seq:
                    for (h, c, _) in USE[t]:
                        self.left[h, c] = self.left.get((h, c), 0) + 1

            def blk(self, k, c):
                if (k, c) not in self.blocks:
                    self.blocks[k, c] = t_rows(2 * self.d + self.fg[c - 1], (k - 1) * KH, KH,
                                               self.prods, self.cell)
                return self.blocks[k, c]

            def rem(self, X):
                if X not in self.rems:
                    ts = t_rows(2 * self.d + X, KM, KR, self.prods, self.cell)
                    tl, tr = (t_rows(2 * self.d + k, KM, KR, (5,) if X else (0,), self.cell)[0]
                              for k in range(2))
                    ce, lo = (b * b * D, -b * D) if self.prods == (1, 2) else (-a * a * D, a * D)
                    if X == 0:
                        e, o = ce * tl, lo * tr
                        zs = (e - o, e + o)
                    else:
                        e, o = (-ce) * tl, lo * tr
                        zs = (e + o, e - o)
                    self.rems[X] = [to_bf16(jnp.concatenate([t, z], axis=0), 8 * i + 7, 2 * KR * X)
                                    for i, t, z in zip(self.prods, ts, zs)]
                return self.rems[X]

            def rhs(self, t, n):
                if (t, n) not in self.rhss:
                    vs = [self.blk(k, c)[n] for (k, c, _) in SDEF[t]]
                    if len(vs) == 2:
                        vs = [vs[0] + vs[1] if SDEF[t][1][2] > 0 else vs[0] - vs[1]]
                    self.rhss[t, n] = to_bf16(vs[0], 8 * self.prods[n] + t - 1, 0)
                return self.rhss[t, n]

            def term(self, t):
                self.todo.remove(t)
                for n, i in enumerate(self.prods):
                    if t < 10:
                        l = jnp.concatenate([a32[i, t - 1, 0], a32[i, t - 1, 1]], axis=1)
                        v = _dot(l, self.rhs(t, n))
                    else:
                        h, X = t // 10 - 1, self.fg[t % 10 - 1]
                        v = _dot(r32[2 * i - 2 + X, h * MH // 2:(h + 1) * MH // 2, :], self.rem(X)[n])
                    for (h, c, sg) in USE[t]:
                        k = (i, h, c)
                        if k not in self.acc:
                            self.acc[k] = (v, sg)
                        else:
                            p, ps = self.acc[k]
                            self.acc[k] = ((p + v, sg) if ps == sg
                                           else (p - v if ps > 0 else v - p, 1))
                for (h, c, _) in USE[t]:
                    self.left[h, c] -= 1
                    if self.left[h, c] == 0:
                        self.ready.append((h, c))

            def flush(self):
                for (h, c) in self.ready:
                    self.on_final(self.fg[c], h, [self.acc[i, h, c][0] for i in self.prods])
                self.ready = []

            def run(self):
                self.flush()
                for t in list(self.todo):
                    self.term(t)
                    self.flush()

        def bias(k, h):
            return sh_ref[k, h * MH:(h + 1) * MH, :]

        for d in range(ND):
            st12, y0p, y3p = {}, {}, {}

            def fin12(X, h, v):
                st12[X, h] = ((v[0] + v[1]) + bias(1, h), a * (v[0] - v[1]) + bias(0, h))

            def fin34(X, h, v):
                p, q = st12[X, h]
                r, s = v[0] + v[1], b * (v[0] - v[1])
                o_ref[8 * d + 4 * X + 1, h * MH:(h + 1) * MH, :] = _silu2(q + s)
                o_ref[8 * d + 4 * X + 2, h * MH:(h + 1) * MH, :] = _silu2((a * a) * p + (b * b) * r)
                y0p[X, h] = p + r
                y3p[X, h] = (a * a) * q + (b * b) * s

            def fin_last(yp, off, kb):
                def f(X, h, v):
                    slab = 8 * d + 4 * X + off
                    y = yp[X, h] + (v[0] + bias(kb, h))
                    if (off == 3) == (X == 0):
                        y = y + shared[h]
                    o_ref[slab, h * MH:(h + 1) * MH, :] = _silu2(y)
                    if d == ND - 1 and (slab, h) not in LATE:
                        out_half(step, slab, h).start()
                return f

            shared = []
            g12 = Group(d, (1, 2), 0, SEQ_12, fin12)
            g34 = Group(d, (3, 4), 1, SEQ_34, fin34)
            g0 = Group(d, (0,), 2, SEQ_05, fin_last(y0p, 0, 2))
            g5 = Group(d, (5,), 3, SEQ_05, fin_last(y3p, 3, 3))
            if first and d == 0:
                for grp in (g12, g34, g5):
                    for t in ((5, 3) if grp.fg[0] else (2, 4)):
                        grp.term(t)
                g0.rhs(2, 0)
                g0.rhs(4, 0)
                wrem_copy.wait()
                fcs[1].wait()
                remainder_lhs()
                g0.term(2)
                g0.term(4)
            if d % 2:
                g0.term(SEQ_05[0])
            g12.run()
            if first and d < 2:
                t = [t for t in g34.todo if t < 10][0]
                g34.todo.remove(t)
                g34.todo.insert(0, t)
                g34.rhs(t, 0)
                g34.rhs(t, 1)
                fcs[2 + d].wait()
            g34.run()
            if d == ND - 1:
                out_copy(step, 8 * d + 1, 2).start()
                out_copy(step, 8 * d + 5, 2).start()
            t = jnp.concatenate([t_rows(2 * d, KM, KR, (5,), 3)[0],
                                 t_rows(2 * d + 1, KM, KR, (0,), 3)[0]], axis=0)
            t = to_bf16(t, 7, 0)
            for h in range(2):
                shared.append(_dot(r32[8, h * MH // 2:(h + 1) * MH // 2, :], t))
            g5.run()
            g0.run()
            if d < ND - 1:
                out_copy(step, 8 * d, 8).start()
            if d == 0 and not first:
                for slab, h in LATE:
                    out_half(step - 1, slab, h).start()

    def scoped_block(step):
        pl.run_scoped(lambda s_ref: block(step, s_ref), pltpu.VMEM((48, KH, TB), bf16))

    scoped_block(0)

    def body(step, carry):
        in_copy(step).wait()

        @pl.when(step >= 2)
        def _():
            out_wait_all(_sl(step))

        @pl.when(step + 1 < NS)
        def _():
            in_copy(step + 1).start()

        scoped_block(step)
        return carry

    jax.lax.fori_loop(1, NS, body, 0)
    for slab, h in LATE:
        out_half(NS - 1, slab, h).start()
    out_wait_all(NS % 2)
    out_wait_all((NS - 1) % 2)


@jax.jit
def pallas_standalone__batchnorm__sampling_kernel(
    x: jax.Array,
    w: jax.Array,
    mean: jax.Array,
    var: jax.Array,
    g: jax.Array,
    b: jax.Array,
):
    B, S, C = x.shape
    xt = jnp.transpose(x, (1, 2, 0))
    out = pl.pallas_call(
        _kernel,
        in_specs=[pl.BlockSpec(memory_space=pl.ANY)] * 6,
        out_specs=pl.BlockSpec(memory_space=pl.ANY),
        out_shape=jax.ShapeDtypeStruct((S, C, B), x.dtype),
        scratch_shapes=[pltpu.VMEM((3, C, C), bf16)] + [pltpu.VMEM((C,), bf16)] * 4 + [
            pltpu.VMEM((6, 7, 2, C // 2, 128), bf16),
            pltpu.VMEM((9, C, 128), bf16),
            pltpu.VMEM((4, C, 128), f32),
            pltpu.VMEM((4, C, 128), f32),
            pltpu.VMEM((2, S, C, TB), bf16),
            pltpu.VMEM((2, S, C, TB), bf16),
            pltpu.SMEM((4,), jnp.int32),
            pltpu.SemaphoreType.DMA((NSEM,)),
        ],
        compiler_params=pltpu.CompilerParams(
            vmem_limit_bytes=100 * 1024 * 1024,
            disable_bounds_checks=True,
            disable_semaphore_checks=True,
        ),
    )(xt, w, mean, var, g, b)
    return jnp.transpose(out, (2, 0, 1))
```

```python
import jax
import jax.numpy as jnp
import jax.experimental.pallas as pl
import jax.experimental.pallas.tpu as pltpu

f32 = jnp.float32
bf16 = jnp.bfloat16
u32 = jnp.uint32

A = 0.6875
Bp = 1.0 / A
TB = 128
KM = 512
KH = KM // 2
RS = 96
SWAP = (0, 1, 1, 0, 0, 1)
SDEF = {1: ((1, 1, 1), (2, 2, 1)), 2: ((1, 1, 1),), 3: ((1, 2, 1), (2, 2, -1)),
        4: ((2, 1, 1), (1, 1, -1)), 5: ((2, 2, 1),), 6: ((1, 1, 1), (1, 2, 1)),
        7: ((2, 1, 1), (2, 2, 1))}
USE = {1: ((0, 0, 1), (1, 1, 1)), 2: ((1, 0, 1), (1, 1, -1)), 3: ((0, 1, 1), (1, 1, 1)),
       4: ((0, 0, 1), (1, 0, 1)), 5: ((0, 0, -1), (0, 1, 1)), 6: ((1, 1, 1),), 7: ((0, 0, 1),),
       11: ((0, 0, 1),), 21: ((1, 0, 1),), 12: ((0, 1, 1),), 22: ((1, 1, 1),)}
SEQ_12 = (2, 4, 21, 12, 5, 3, 22, 11, 1, 6, 7)
SEQ_34 = (2, 4, 21, 12, 5, 3, 1, 22, 11, 6, 7)
SEQ_05 = (2, 4, 5, 3, 1, 6, 7)
FIRST = ((0, 5), (5, 9), (9, 17), (17, 32))
LATE = ((28, 1), (24, 0))
PS, WS, FS = 0, 4, 9
IS = FS + len(FIRST)
OS = IS + 2
NSEM = OS + 2


def _upk(v):
    return pltpu.bitcast(v, bf16)


def _dsm(lo, n):
    return pl.ds(lo if isinstance(lo, int) else pl.multiple_of(lo, n), n)


def _sl(st):
    return st % 2 if isinstance(st, int) else st & 1


def _silu2(h):
    return (h + h * jnp.tanh(h)).astype(bf16)


def _dot(l, r):
    return jnp.dot(_upk(l), r, preferred_element_type=f32)


def _kernel(x_hbm, w_hbm, m_hbm, v_hbm, g_hbm, b_hbm, o_hbm,
            wbuf, pm, pv, pg, pb, a_ref, r_ref, sc_ref, sh_ref, xbuf, obuf, z_ref, sem):
    S, C, B = x_hbm.shape
    ND = S // 8
    NS = B // TB
    MH = C // 2
    KR = C - KM
    a, b = A, Bp
    cc = a * a + b * b
    D = 1.0 / (2 * (b * b - a * a))
    a32, r32 = a_ref.bitcast(u32), r_ref.bitcast(u32)

    def x_copy(st, lo, hi, s):
        return pltpu.make_async_copy(
            x_hbm.at[pl.ds(lo, hi - lo), :, _dsm(st * TB, TB)],
            xbuf.at[_sl(st), pl.ds(lo, hi - lo)], s)

    def in_copy(st):
        return x_copy(st, 0, S, sem.at[IS + _sl(st)])

    def out_copy(st, lo, n):
        return pltpu.make_async_copy(
            obuf.at[_sl(st), pl.ds(lo, n)],
            o_hbm.at[pl.ds(lo, n), :, _dsm(st * TB, TB)], sem.at[OS + _sl(st)])

    def out_half(st, slab, h):
        return pltpu.make_async_copy(
            obuf.at[_sl(st), slab, pl.ds(h * MH, MH)],
            o_hbm.at[slab, pl.ds(h * MH, MH), _dsm(st * TB, TB)], sem.at[OS + _sl(st)])

    def out_wait_all(sl):
        pltpu.make_async_copy(obuf.at[sl], obuf.at[sl], sem.at[OS + sl]).wait()

    pcs = [pltpu.make_async_copy(s, d, sem.at[PS + i])
           for i, (s, d) in enumerate(((m_hbm, pm), (v_hbm, pv), (g_hbm, pg), (b_hbm, pb)))]

    def w_copy(r):
        return pltpu.make_async_copy(w_hbm.at[:, _dsm(r * 128, 128), :],
                                     wbuf.at[:, _dsm(r * 128, 128), :], sem.at[WS + r])

    wrem_copy = pltpu.make_async_copy(w_hbm.at[:, pl.ds(KM, KR), :],
                                      wbuf.at[:, pl.ds(KM, KR), :], sem.at[WS + 4])
    fcs = [x_copy(0, lo, hi, sem.at[FS + k]) for k, (lo, hi) in enumerate(FIRST)]

    def u_vals(gs, lo, n):
        sc = [sc_ref[k, lo:lo + n, :] for k in range(4)]
        u0 = gs[0] * sc[0]
        u5 = gs[2] * sc[1]
        e = D * u5
        ea = (b * b * D) * u0 - e
        eb = e - (a * a * D) * u0
        hb = gs[1] * sc[2]
        ha = gs[1] * sc[3]
        return [u0, ea - hb, ea + hb, eb + ha, eb - ha, u5]

    eye = (jax.lax.broadcasted_iota(jnp.int32, (128, 128), 0)
           == jax.lax.broadcasted_iota(jnp.int32, (128, 128), 1)).astype(f32).astype(bf16)

    def tr_rows(k, q, lo, n):
        out = []
        while n > 0:
            t, o = lo // 128, lo % 128
            m = min(n, 128 - o)
            wd = min(128, C - 128 * t)
            w = wbuf[k, _dsm(q * 128, 128), 128 * t:128 * t + wd]
            out.append(jax.lax.dot_general(eye[o:o + m, :wd], w, (((1,), (1,)), ((), ())),
                                           preferred_element_type=f32))
            lo, n = lo + m, n - m
        return out[0] if len(out) == 1 else jnp.concatenate(out, axis=0)

    def strassen_lhs(r, carry):
        z_ref[r] = 0
        z_ref[r + 2] = 0
        w_copy(r).wait()
        w_copy(r + 2).wait()
        for c in range(MH // RS):
            us = {}
            for h in range(2):
                lo = h * MH + c * RS
                gs = [[tr_rows(k, r + 2 * q, lo, RS) for k in range(3)] for q in range(2)]
                for q in range(2):
                    us[h, q] = u_vals(gs[q], lo, RS)
            for i in range(6):
                a11, a12, a21, a22 = us[0, 0][i], us[0, 1][i], us[1, 0][i], us[1, 1][i]
                for s, v in enumerate((a11 + a22, a21 + a22, a11, a22,
                                       a11 + a12, a21 - a11, a12 - a22)):
                    a_ref[i, s, r, c * RS:(c + 1) * RS, :] = v.astype(bf16)
        return carry

    def remainder_lhs():
        wr = [wbuf[k, KM:, :] for k in range(3)]
        us = u_vals([jnp.concatenate([w, w], axis=0).T.astype(f32) for w in wr], 0, C)
        low = jax.lax.broadcasted_iota(jnp.int32, (C, 2 * KR), 1) < KR
        for i in range(1, 5):
            r_ref[2 * i - 2] = jnp.where(low, us[i], us[0]).astype(bf16)
            r_ref[2 * i - 1] = jnp.where(low, us[i], us[5]).astype(bf16)
        r_ref[8] = jnp.where(low, us[5], us[0]).astype(bf16)

    for c in pcs + [w_copy(r) for r in (0, 2, 1, 3)] + [fcs[0], wrem_copy] + fcs[1:]:
        c.start()
    in_copy(1).start()
    for c in pcs:
        c.wait()
    mean, var, g, bb = (r[...].reshape(1, C).astype(f32) for r in (pm, pv, pg, pb))
    sc_all = 0.5 * g / jnp.sqrt(var + 1e-5)
    scc = jnp.broadcast_to(sc_all, (128, C)).T
    sc_ref[0] = -scc
    sc_ref[1] = scc
    sc_ref[2] = (b * D) * scc
    sc_ref[3] = (a * D) * scc
    sh = jnp.broadcast_to(0.5 * bb - mean * sc_all, (128, C)).T
    sh_ref[0] = sh
    sh_ref[1] = (b * b) * sh
    sh_ref[2] = (1.0 - b * b) * sh
    sh_ref[3] = (1.0 - a * a) * sh
    jax.lax.fori_loop(0, 2, strassen_lhs, 0)
    fcs[0].wait()

    def block(step, s_ref):
        first = isinstance(step, int)
        o_ref = obuf.at[_sl(step)]
        s32 = s_ref.bitcast(u32)

        def t_rows(j, lo, n, grp, cell):
            xb = xbuf.at[(step + z_ref[cell]) & 1]

            def dd(k):
                i = 4 * j - 1 + k
                return xb[i, lo:lo + n, :].astype(f32) if 0 <= i < S else None

            if grp == (1, 2):
                p = dd(4) - (b * b) * dd(2)
                q = a * dd(3) - b * dd(1)
                return p + q, p - q
            if grp == (3, 4):
                p = dd(4) - (a * a) * dd(2)
                q = b * dd(3) - a * dd(1)
                return p + q, p - q
            if grp == (0,):
                d0 = dd(0)
                return (cc * dd(2) - (dd(4) if d0 is None else dd(4) + d0),)
            d5 = dd(5)
            return ((dd(1) if d5 is None else dd(1) + d5) - cc * dd(3),)

        def to_bf16(v, e, lo):
            n = v.shape[0]
            s_ref[e, lo:lo + n, :] = v.astype(bf16)
            return _upk(s32[e, lo // 2:(lo + n) // 2, :])

        class Group:
            def __init__(self, d, prods, cell, seq, on_final):
                self.d, self.prods, self.cell, self.on_final = d, prods, cell, on_final
                self.fg = (1, 0) if SWAP[prods[0]] else (0, 1)
                self.todo = list(seq)
                self.blocks, self.rems, self.rhss = {}, {}, {}
                self.acc, self.left, self.ready = {}, {}, []
                for t in seq:
                    for (h, c, _) in USE[t]:
                        self.left[h, c] = self.left.get((h, c), 0) + 1

            def blk(self, k, c):
                if (k, c) not in self.blocks:
                    self.blocks[k, c] = t_rows(2 * self.d + self.fg[c - 1], (k - 1) * KH, KH,
                                               self.prods, self.cell)
                return self.blocks[k, c]

            def rem(self, X):
                if X not in self.rems:
                    ts = t_rows(2 * self.d + X, KM, KR, self.prods, self.cell)
                    tl, tr = (t_rows(2 * self.d + k, KM, KR, (5,) if X else (0,), self.cell)[0]
                              for k in range(2))
                    ce, lo = (b * b * D, -b * D) if self.prods == (1, 2) else (-a * a * D, a * D)
                    if X == 0:
                        e, o = ce * tl, lo * tr
                        zs = (e - o, e + o)
                    else:
                        e, o = (-ce) * tl, lo * tr
                        zs = (e + o, e - o)
                    self.rems[X] = [to_bf16(jnp.concatenate([t, z], axis=0), 8 * i + 7, 2 * KR * X)
                                    for i, t, z in zip(self.prods, ts, zs)]
                return self.rems[X]

            def rhs(self, t, n):
                if (t, n) not in self.rhss:
                    vs = [self.blk(k, c)[n] for (k, c, _) in SDEF[t]]
                    if len(vs) == 2:
                        vs = [vs[0] + vs[1] if SDEF[t][1][2] > 0 else vs[0] - vs[1]]
                    self.rhss[t, n] = to_bf16(vs[0], 8 * self.prods[n] + t - 1, 0)
                return self.rhss[t, n]

            def term(self, t):
                self.todo.remove(t)
                for n, i in enumerate(self.prods):
                    if t < 10:
                        l = jnp.concatenate([a32[i, t - 1, 0], a32[i, t - 1, 1]], axis=1)
                        v = _dot(l, self.rhs(t, n))
                    else:
                        h, X = t // 10 - 1, self.fg[t % 10 - 1]
                        v = _dot(r32[2 * i - 2 + X, h * MH // 2:(h + 1) * MH // 2, :], self.rem(X)[n])
                    for (h, c, sg) in USE[t]:
                        k = (i, h, c)
                        if k not in self.acc:
                            self.acc[k] = (v, sg)
                        else:
                            p, ps = self.acc[k]
                            self.acc[k] = ((p + v, sg) if ps == sg
                                           else (p - v if ps > 0 else v - p, 1))
                for (h, c, _) in USE[t]:
                    self.left[h, c] -= 1
                    if self.left[h, c] == 0:
                        self.ready.append((h, c))

            def flush(self):
                for (h, c) in self.ready:
                    self.on_final(self.fg[c], h, [self.acc[i, h, c][0] for i in self.prods])
                self.ready = []

            def run(self):
                self.flush()
                for t in list(self.todo):
                    self.term(t)
                    self.flush()

        def bias(k, h):
            return sh_ref[k, h * MH:(h + 1) * MH, :]

        for d in range(ND):
            st12, y0p, y3p = {}, {}, {}

            def fin12(X, h, v):
                st12[X, h] = ((v[0] + v[1]) + bias(1, h), a * (v[0] - v[1]) + bias(0, h))

            def fin34(X, h, v):
                p, q = st12[X, h]
                r, s = v[0] + v[1], b * (v[0] - v[1])
                o_ref[8 * d + 4 * X + 1, h * MH:(h + 1) * MH, :] = _silu2(q + s)
                o_ref[8 * d + 4 * X + 2, h * MH:(h + 1) * MH, :] = _silu2((a * a) * p + (b * b) * r)
                y0p[X, h] = p + r
                y3p[X, h] = (a * a) * q + (b * b) * s

            def fin_last(yp, off, kb):
                def f(X, h, v):
                    slab = 8 * d + 4 * X + off
                    y = yp[X, h] + (v[0] + bias(kb, h))
                    if (off == 3) == (X == 0):
                        y = y + shared[h]
                    o_ref[slab, h * MH:(h + 1) * MH, :] = _silu2(y)
                    if d == ND - 1 and (slab, h) not in LATE:
                        out_half(step, slab, h).start()
                return f

            shared = []

            def shared_tile():
                if not shared:
                    t = jnp.concatenate([t_rows(2 * d, KM, KR, (5,), 3)[0],
                                         t_rows(2 * d + 1, KM, KR, (0,), 3)[0]], axis=0)
                    t = to_bf16(t, 7, 0)
                    for h in range(2):
                        shared.append(_dot(r32[8, h * MH // 2:(h + 1) * MH // 2, :], t))

            g12 = Group(d, (1, 2), 0, SEQ_12, fin12)
            g34 = Group(d, (3, 4), 1, SEQ_34, fin34)
            g0 = Group(d, (0,), 2, SEQ_05, fin_last(y0p, 0, 2))
            g5 = Group(d, (5,), 3, SEQ_05, fin_last(y3p, 3, 3))
            if first and d == 0:
                for grp in (g12, g34, g5):
                    for t in ((5, 3) if grp.fg[0] else (2, 4)):
                        grp.term(t)
                g0.rhs(2, 0)
                g0.rhs(4, 0)
                wrem_copy.wait()
                fcs[1].wait()
                remainder_lhs()
                g0.term(2)
                g0.term(4)
            if d == 0 and not first:
                shared_tile()
            if d % 2 or (d == 0 and not first):
                g0.term(SEQ_05[0])
            g12.run()
            if first and d < 2:
                t = [t for t in g34.todo if t < 10][0]
                g34.todo.remove(t)
                g34.todo.insert(0, t)
                g34.rhs(t, 0)
                g34.rhs(t, 1)
                fcs[2 + d].wait()
            g34.run()
            if d == ND - 1:
                out_copy(step, 8 * d + 1, 2).start()
                out_copy(step, 8 * d + 5, 2).start()
            shared_tile()
            g5.run()
            g0.run()
            if d < ND - 1:
                out_copy(step, 8 * d, 8).start()
            if d == 0 and not first:
                for slab, h in LATE:
                    out_half(step - 1, slab, h).start()

    def scoped_block(step):
        pl.run_scoped(lambda s_ref: block(step, s_ref), pltpu.VMEM((48, KH, TB), bf16))

    scoped_block(0)

    def body(step, carry):
        in_copy(step).wait()

        @pl.when(step >= 2)
        def _():
            out_wait_all(_sl(step))

        @pl.when(step + 1 < NS)
        def _():
            in_copy(step + 1).start()

        scoped_block(step)
        return carry

    jax.lax.fori_loop(1, NS, body, 0)
    for slab, h in LATE:
        out_half(NS - 1, slab, h).start()
    out_wait_all(NS % 2)
    out_wait_all((NS - 1) % 2)


@jax.jit
def pallas_standalone__batchnorm__sampling_kernel(
    x: jax.Array,
    w: jax.Array,
    mean: jax.Array,
    var: jax.Array,
    g: jax.Array,
    b: jax.Array,
):
    B, S, C = x.shape
    xt = jnp.transpose(x, (1, 2, 0))
    out = pl.pallas_call(
        _kernel,
        in_specs=[pl.BlockSpec(memory_space=pl.ANY)] * 6,
        out_specs=pl.BlockSpec(memory_space=pl.ANY),
        out_shape=jax.ShapeDtypeStruct((S, C, B), x.dtype),
        scratch_shapes=[pltpu.VMEM((3, C, C), bf16)] + [pltpu.VMEM((C,), bf16)] * 4 + [
            pltpu.VMEM((6, 7, 2, C // 2, 128), bf16),
            pltpu.VMEM((9, C, 128), bf16),
            pltpu.VMEM((4, C, 128), f32),
            pltpu.VMEM((4, C, 128), f32),
            pltpu.VMEM((2, S, C, TB), bf16),
            pltpu.VMEM((2, S, C, TB), bf16),
            pltpu.SMEM((4,), jnp.int32),
            pltpu.SemaphoreType.DMA((NSEM,)),
        ],
        compiler_params=pltpu.CompilerParams(
            vmem_limit_bytes=100 * 1024 * 1024,
            disable_bounds_checks=True,
            disable_semaphore_checks=True,
        ),
    )(xt, w, mean, var, g, b)
    return jnp.transpose(out, (2, 0, 1))
```
